```python
import jax
import jax.numpy as jnp

def _softmax(x, axis=-1):
    return jax.nn.softmax(x, axis=axis)
def _gelu(x):
    return jax.nn.gelu(x, approximate=True)
def _silu(x):
    return jax.nn.silu(x)
def _sigmoid(x):
    return jax.nn.sigmoid(x)
def _layernorm(x, axis=-1, eps=1e-5):
    m = jnp.mean(x, axis=axis, keepdims=True)
    v = jnp.var(x, axis=axis, keepdims=True)
    return (x - m) / jnp.sqrt(v + eps)
def _scatter_add(tgt, idx, src, axis=0):
    return tgt.at[idx].add(src)
def _segment_sum(src, seg, n):
    return jax.ops.segment_sum(src, seg, n)
class _Rng:
    def __init__(self, key):
        self._k = key
    def _next(self):
        self._k, sub = jax.random.split(self._k)
        return sub
    def normal(self, shape):
        return jax.random.normal(self._next(), shape, dtype=jnp.bfloat16)
    def randint(self, lo, hi, shape):
        return jax.random.randint(self._next(), shape, lo, hi, dtype=jnp.int32)
    def uniform(self, shape, lo=0.0, hi=1.0):
        return jax.random.uniform(self._next(), shape, jnp.bfloat16, lo, hi)
    def permutation(self, n):
        return jax.random.permutation(self._next(), n)


kernel_name = 'interleave_layers__sliding_local_dilated__dense_activation_gelu__prompt'

def setup_inputs():
    _rng = _Rng(jax.random.key(int.from_bytes(__import__("os").urandom(4), "little")))
    _w = (lambda a: (lambda t: t.astype(jnp.bfloat16) if jnp.issubdtype(t.dtype, jnp.floating) else t)(jnp.asarray(a)))
    def _A_setup():
        B, S, D = 1, 2048, 1024
        return {
            "x": _w((lambda *s: _rng.normal(s) * 0.05)(B, S, D)),
            "wqkv": _w((lambda *s: _rng.normal(s) * 0.05)(D, 3 * D)),
            "wo": _w((lambda *s: _rng.normal(s) * 0.05)(D, D)),
        }
    _A_in = _A_setup()

    def _B_setup():
        B, S, D, F = 1, 2048, 1024, 3584
        return {
            "x": _w((lambda *s: _rng.normal(s) * 0.05)(B, S, D)),
            "w1": _w((lambda *s: _rng.normal(s) * 0.05)(D, F) * (D ** -0.5)),
            "b1": _w((lambda *s: _rng.normal(s) * 0.05)(F) * 0.01),
            "w2": _w((lambda *s: _rng.normal(s) * 0.05)(F, D) * (F ** -0.5)),
            "b2": _w((lambda *s: _rng.normal(s) * 0.05)(D) * 0.01),
        }
    _B_in = _B_setup()

    return {
        "A_x": _A_in["x"],
        "A_wqkv": _A_in["wqkv"],
        "A_wo": _A_in["wo"],
        "B_x": _B_in["x"],
        "B_w1": _B_in["w1"],
        "B_b1": _B_in["b1"],
        "B_w2": _B_in["w2"],
        "B_b2": _B_in["b2"],
    }

def reference(A_x, A_wqkv, A_wo, B_x, B_w1, B_b1, B_w2, B_b2):
    def _A_ref(x, wqkv, wo):
        B, S, D = x.shape
        H = 32; Dh = D // H
        W, dil = 8, 2
        qkv = (lambda x, *d: x.transpose(*d))((x @ wqkv).reshape(B, S, 3, H, Dh), 2, 0, 3, 1, 4)
        q, k, v = qkv[0], qkv[1], qkv[2]
        scale = Dh ** -0.5
        pos = jnp.arange(S)
        off = jnp.arange(W) * dil
        idx = pos[:, None] - off[None, :]
        mask = idx >= 0
        idx_c = jnp.where(mask, idx, 0).reshape(-1)
        kg = k[:, :, idx_c, :].reshape(B, H, S, W, Dh)
        vg = v[:, :, idx_c, :].reshape(B, H, S, W, Dh)
        logits = jnp.einsum("bhsd,bhswd->bhsw", q, kg) * scale
        logits = jnp.where(mask[None, None, :, :], logits, -1e9)
        attn = _softmax(logits, axis=-1)
        o = jnp.einsum("bhsw,bhswd->bhsd", attn, vg)
        return (lambda x, *d: x.transpose(*d))(o, 0, 2, 1, 3).reshape(B, S, D) @ wo

    def _B_ref(x, w1, b1, w2, b2):
        h = jnp.einsum("bsd,df->bsf", x, w1) + b1
        h = _gelu(h)
        return jnp.einsum("bsf,fd->bsd", h, w2) + b2

    x = A_x
    x = x + _A_ref(_layernorm(x, axis=-1), A_wqkv, A_wo)
    x = x + _B_ref(_layernorm(x, axis=-1), B_w1, B_b1, B_w2, B_b2)
    x = x + _A_ref(_layernorm(x, axis=-1), A_wqkv, A_wo)
    x = x + _B_ref(_layernorm(x, axis=-1), B_w1, B_b1, B_w2, B_b2)
    return x
```

```python
import functools

import jax
import jax.numpy as jnp
import jax.experimental.pallas as pl
import jax.experimental.pallas.tpu as pltpu

S, D, F = 2048, 1024, 3584
H, DH, WIN, DIL = 32, 32, 8, 2
NC = D // 128
HALO = 16
EPS = 1e-5
F32, BF16 = jnp.float32, jnp.bfloat16
NT = (((1,), (1,)), ((), ()))


def _ln(x):
    m = jnp.mean(x, axis=-1, keepdims=True)
    xc = x - m
    v = jnp.mean(xc * xc, axis=-1, keepdims=True)
    return (xc * jax.lax.rsqrt(v + EPS)).astype(BF16)


def _gelu(x):
    c = 0.7978845608028654
    t = jnp.tanh(x * (c + (c * 0.044715) * (x * x)))
    hx = 0.5 * x
    return hx + hx * t


def _kernel(x_ref, wqkv_hbm, wo_hbm, w1_hbm, b1_ref, w2_hbm, b2_ref, o_ref,
            wq_raw, wo_raw, wt, wo_p, w1, w2, tmp, xs, x1_s, y_s, q_s, k_s, v_s, o_s, sems,
            *, TM, FC, RC):
    NB = S // TM
    s = pl.program_id(0)
    NFC = F // FC
    NRC = TM // RC

    def attn_front(first):
        if first:
            xc = x_ref[...].astype(F32)
            xs[0:TM, :] = xc
        else:
            row0 = pl.multiple_of((s % NB) * TM, TM)
            xc = jnp.where(s < NB, x_ref[...].astype(F32), xs[pl.ds(row0, TM), :])
            xs[pl.ds(row0, TM), :] = xc
        return _ln(xc)

    def halo(first):
        for buf in (k_s, v_s):
            if first:
                buf[:, 0:HALO, :] = jnp.zeros((NC, HALO, 128), F32)
            else:
                buf[:, 0:HALO, :] = buf[:, TM:TM + HALO, :]

    def proj(xn, t):
        dst, off = ((q_s, 0), (k_s, HALO), (v_s, HALO))[t]
        r = jax.lax.dot_general(xn, wt[t * D:(t + 1) * D, :], NT, preferred_element_type=F32)
        for c in range(NC):
            dst[c, off:off + TM, :] = r[:, c * 128:(c + 1) * 128]

    def attn_rows(r):
        r0 = r * RC
        q = [q_s[c, r0:r0 + RC, :] for c in range(NC)]
        lg = []
        for w in range(WIN):
            a = r0 + HALO - DIL * w
            p = [q[c] * k_s[c, a:a + RC, :] for c in range(NC)]
            t = ((p[0] + p[1]) + (p[2] + p[3])) + ((p[4] + p[5]) + (p[6] + p[7]))
            t = t + pltpu.roll(t, 64, 1)
            t = t + pltpu.roll(t, 32, 1)
            t = t * (DH ** -0.5)
            if w > 0 and r0 < DIL * w:
                pos = (s % NB) * TM + r0 + jax.lax.broadcasted_iota(jnp.int32, (RC, 128), 0)
                t = jnp.where(pos >= DIL * w, t, -1e9)
            lg.append(t)
        m = functools.reduce(jnp.maximum, lg)
        e = [jnp.exp(t - m) for t in lg]
        den = ((e[0] + e[1]) + (e[2] + e[3])) + ((e[4] + e[5]) + (e[6] + e[7]))
        inv = 1.0 / den
        e = [t * inv for t in e]
        for c in range(NC):
            p = [e[w] * v_s[c, r0 + HALO - DIL * w:r0 + HALO - DIL * w + RC, :] for w in range(WIN)]
            t = ((p[0] + p[1]) + (p[2] + p[3])) + ((p[4] + p[5]) + (p[6] + p[7]))
            o_s[r0:r0 + RC, c * 128:(c + 1) * 128] = t.astype(BF16)

    def out_proj():
        prow = pl.multiple_of(((s - 1) % NB) * TM, TM)
        x1 = xs[pl.ds(prow, TM), :] + jnp.dot(o_s[...], wo_p[...], preferred_element_type=F32)
        x1_s[...] = x1 + b2_ref[...].astype(F32)
        y_s[...] = _ln(x1)

    def mlp(with_attn):
        done = 0
        for c in range(NFC):
            h = jnp.dot(y_s[...], w1[:, c * FC:(c + 1) * FC], preferred_element_type=F32)
            h = _gelu(h + b1_ref[:, c * FC:(c + 1) * FC].astype(F32)).astype(BF16)
            acc = x1_s[...] + jnp.dot(h, w2[c * FC:(c + 1) * FC, :], preferred_element_type=F32)
            if c < NFC - 1:
                x1_s[...] = acc
            else:
                prow = pl.multiple_of(((s - 1) % NB) * TM, TM)
                xs[pl.ds(prow, TM), :] = acc
                o_ref[...] = acc.astype(BF16)
            if with_attn:
                upto = min(NRC, -(-NRC * (c + 1) // (NFC - 1)))
                for r in range(done, upto):
                    attn_rows(r)
                done = upto

    def copies():
        cq = [pltpu.make_async_copy(wqkv_hbm.at[:, t * D:(t + 1) * D], wq_raw.at[t], sems.at[t])
              for t in range(3)]
        return cq + [pltpu.make_async_copy(wo_hbm, wo_raw, sems.at[3]),
                     pltpu.make_async_copy(w1_hbm, w1, sems.at[4]),
                     pltpu.make_async_copy(w2_hbm, w2, sems.at[5])]

    def permute_from_tmp(dst, base):
        for kc in range(NC):
            for d in range(DH):
                dst[base + d * H:base + (d + 1) * H, kc * 128:(kc + 1) * 128] = (
                    tmp[kc, pl.ds(d, H, stride=DH), :].astype(BF16))

    @pl.when(s == 0)
    def _prologue():
        cps = copies()
        for cp in cps:
            cp.start()
        xn = attn_front(True)
        halo(True)
        o_ref[...] = jnp.zeros(o_ref.shape, BF16)
        eye = (jax.lax.broadcasted_iota(jnp.int32, (128, 128), 0)
               == jax.lax.broadcasted_iota(jnp.int32, (128, 128), 1)).astype(BF16)
        for t in range(3):
            cps[t].wait()
            for c in range(NC):
                tile = jax.lax.dot_general(eye, wq_raw[t, :, c * 128:(c + 1) * 128], NT,
                                           preferred_element_type=F32)
                for kc in range(NC):
                    tmp[kc, c * 128:(c + 1) * 128, :] = tile[:, kc * 128:(kc + 1) * 128]
            permute_from_tmp(wt, t * D)
            proj(xn, t)
        cps[3].wait()
        for kc in range(NC):
            tmp[kc] = wo_raw[:, kc * 128:(kc + 1) * 128].astype(F32)
        permute_from_tmp(wo_p, 0)
        for r in range(NRC):
            attn_rows(r)
        cps[4].wait()
        cps[5].wait()

    @pl.when(jnp.logical_and(s > 0, s < 2 * NB))
    def _main():
        out_proj()
        xn = attn_front(False)
        halo(False)
        for t in range(3):
            proj(xn, t)
        mlp(True)

    @pl.when(s == 2 * NB)
    def _epilogue():
        out_proj()
        mlp(False)


def _build(TM=256, FC=512, RC=16):
    NB = S // TM
    any_spec = pl.BlockSpec(memory_space=pl.ANY)
    return pl.pallas_call(
        functools.partial(_kernel, TM=TM, FC=FC, RC=RC),
        grid=(2 * NB + 1,),
        in_specs=[
            pl.BlockSpec((TM, D), lambda s: (jnp.minimum(s, NB - 1), 0)),
            any_spec, any_spec, any_spec,
            pl.BlockSpec((1, F), lambda s: (0, 0)),
            any_spec,
            pl.BlockSpec((1, D), lambda s: (0, 0)),
        ],
        out_specs=pl.BlockSpec((TM, D), lambda s: (jnp.maximum(s - 1 - NB, 0), 0)),
        out_shape=jax.ShapeDtypeStruct((S, D), BF16),
        scratch_shapes=[
            pltpu.VMEM((3, D, D), BF16),
            pltpu.VMEM((D, D), BF16),
            pltpu.VMEM((3 * D, D), BF16),
            pltpu.VMEM((D, D), BF16),
            pltpu.VMEM((D, F), BF16),
            pltpu.VMEM((F, D), BF16),
            pltpu.VMEM((NC, D, 128), F32),
            pltpu.VMEM((S, D), F32),
            pltpu.VMEM((TM, D), F32),
            pltpu.VMEM((TM, D), BF16),
            pltpu.VMEM((NC, TM, 128), F32),
            pltpu.VMEM((NC, TM + HALO, 128), F32),
            pltpu.VMEM((NC, TM + HALO, 128), F32),
            pltpu.VMEM((TM, D), BF16),
            pltpu.SemaphoreType.DMA((6,)),
        ],
        compiler_params=pltpu.CompilerParams(
            dimension_semantics=("arbitrary",), vmem_limit_bytes=100 * 1024 * 1024),
    )


@jax.jit
def pallas_interleave_layers__sliding_local_dilated__dense_activation_gelu__prompt_kernel(
    A_x: jax.Array,
    A_wqkv: jax.Array,
    A_wo: jax.Array,
    B_x: jax.Array,
    B_w1: jax.Array,
    B_b1: jax.Array,
    B_w2: jax.Array,
    B_b2: jax.Array,
):
    del B_x
    out = _build()(A_x.reshape(S, D), A_wqkv, A_wo, B_w1, B_b1.reshape(1, F), B_w2,
                   B_b2.reshape(1, D))
    return out.reshape(1, S, D)
```

```python
import functools

import jax
import jax.numpy as jnp
import jax.experimental.pallas as pl
import jax.experimental.pallas.tpu as pltpu

S, D, F = 2048, 1024, 3584
H, DH, WIN, DIL = 32, 32, 8, 2
NC = D // 128
HALO = 16
EPS = 1e-5
PAD = DH + 1
F32, BF16 = jnp.float32, jnp.bfloat16
NT = (((1,), (1,)), ((), ()))


def _ln(x):
    m = jnp.mean(x, axis=-1, keepdims=True)
    xc = x - m
    v = jnp.mean(xc * xc, axis=-1, keepdims=True)
    return (xc * jax.lax.rsqrt(v + EPS)).astype(BF16)


def _gelu(x):
    c = 0.7978845608028654
    t = jnp.tanh(x * (c + (c * 0.044715) * (x * x)))
    hx = 0.5 * x
    return hx + hx * t


def _kernel(x_ref, wqkv_hbm, wo_hbm, w1_hbm, b1_ref, w2_hbm, b2_ref, o_ref,
            wq_raw, wo_raw, wt, wo_p, w1, w2, tmp, xs, x1_s, xn_s, y_s, qkv_s, o_s, sems,
            *, TM, FC, RC, TOK):
    NB = S // TM
    s = pl.program_id(0)
    NFC = F // FC
    NRC = TM // RC
    row0 = pl.multiple_of((s % NB) * TM, TM)
    prow = pl.multiple_of(((s + NB - 1) % NB) * TM, TM)
    live = (jax.lax.broadcasted_iota(jnp.int32, (RC, 128), 0) + s) >= 0

    def ln1(first):
        if first:
            xc = x_ref[...].astype(F32)
        else:
            xc = jnp.where(s < NB, x_ref[...].astype(F32), xs[pl.ds(row0, TM), :])
        xs[pl.ds(row0, TM), :] = xc
        xn_s[...] = _ln(xc)

    def proj(t):
        r = jax.lax.dot_general(xn_s[...], wt[t], NT, preferred_element_type=F32)
        for c in range(NC):
            qkv_s[t, c, HALO:HALO + TM, :] = r[:, c * 128:(c + 1) * 128]

    def tree(p):
        return ((p[0] + p[1]) + (p[2] + p[3])) + ((p[4] + p[5]) + (p[6] + p[7]))

    def attn_rows(r0, masked, tok=None):
        q = [qkv_s[0, c, pl.ds(r0 + HALO, RC), :] for c in range(NC)]
        if tok is not None:
            q = [jnp.where(live, t, tok) for t in q]
        lg = []
        for w in range(WIN):
            a = r0 + HALO - DIL * w
            t = tree([q[c] * qkv_s[1, c, pl.ds(a, RC), :] for c in range(NC)])
            t = t + pltpu.roll(t, 64, 1)
            t = t + pltpu.roll(t, 32, 1)
            t = t * (DH ** -0.5)
            if w > 0 and masked:
                pos = row0 + r0 + jax.lax.broadcasted_iota(jnp.int32, (RC, 128), 0)
                t = jnp.where(pos >= DIL * w, t, -1e9)
            lg.append(t)
        m = jnp.maximum(jnp.maximum(jnp.maximum(lg[0], lg[1]), jnp.maximum(lg[2], lg[3])),
                        jnp.maximum(jnp.maximum(lg[4], lg[5]), jnp.maximum(lg[6], lg[7])))
        e = [jnp.exp(t - m) for t in lg]
        den = tree(e)
        inv = pl.reciprocal(den, approx=True)
        inv = inv * (2.0 - den * inv)
        for c in range(NC):
            t = tree([e[w] * qkv_s[2, c, pl.ds(r0 + HALO - DIL * w, RC), :] for w in range(WIN)])
            o_s[pl.ds(r0, RC), c * 128:(c + 1) * 128] = (t * inv).astype(BF16)

    def out_proj():
        x1 = xs[pl.ds(prow, TM), :] + jnp.dot(o_s[...], wo_p[...], preferred_element_type=F32)
        x1_s[...] = x1

    def ln2():
        y_s[...] = _ln(x1_s[...])

    def mlp_attn():
        g = 0
        for c in range(NFC):
            h = jnp.dot(y_s[...], w1[:, c * FC:(c + 1) * FC], preferred_element_type=F32)
            h = _gelu(h + b1_ref[:, c * FC:(c + 1) * FC].astype(F32)).astype(BF16)
            acc = x1_s[...] + jnp.dot(h, w2[c * FC:(c + 1) * FC, :], preferred_element_type=F32)
            if c < NFC - 1:
                x1_s[...] = acc
            else:
                acc = acc + b2_ref[...].astype(F32)
                xs[pl.ds(prow, TM), :] = acc
                o_ref[...] = acc.astype(BF16)
            n = min(NRC - g, -(-NRC // (NFC - 1)))
            for j in range(n):
                col = (j * NC) // n
                tok = acc[0:RC, col * 128:(col + 1) * 128] if TOK else None
                attn_rows(g * RC, g * RC < HALO, tok)
                g += 1

    def wq_copy(t):
        return pltpu.make_async_copy(wqkv_hbm.at[:, pl.ds(t * D, D)], wq_raw.at[t], sems.at[t])

    wo_copy = pltpu.make_async_copy(wo_hbm, wo_raw, sems.at[3])
    w1_copy = pltpu.make_async_copy(w1_hbm, w1, sems.at[4])
    w2_copy = pltpu.make_async_copy(w2_hbm, w2, sems.at[5])

    def permute_from_tmp(dst):
        for d in range(DH):
            for kc in range(NC):
                dst[d * H:(d + 1) * H, kc * 128:(kc + 1) * 128] = (
                    tmp[kc, pl.ds(d, H, stride=PAD), :].astype(BF16))

    @pl.when(s == 0)
    def _prologue():
        for t in range(3):
            wq_copy(t).start()
        wo_copy.start()
        w1_copy.start()
        w2_copy.start()
        ln1(True)
        qkv_s[:, :, 0:HALO, :] = jnp.zeros((3, NC, HALO, 128), F32)
        o_ref[...] = jnp.zeros(o_ref.shape, BF16)
        eye = (jax.lax.broadcasted_iota(jnp.int32, (128, 128), 0)
               == jax.lax.broadcasted_iota(jnp.int32, (128, 128), 1)).astype(BF16)

        def qkv_body(t, carry):
            wq_copy(t).wait()
            for c in range(NC):
                tile = jax.lax.dot_general(eye, wq_raw[t, :, c * 128:(c + 1) * 128], NT,
                                           preferred_element_type=F32)
                for kc in range(NC):
                    for hh in range(4):
                        tmp[kc, (4 * c + hh) * PAD:(4 * c + hh) * PAD + DH, :] = (
                            tile[hh * DH:(hh + 1) * DH, kc * 128:(kc + 1) * 128])
            permute_from_tmp(wt.at[t])
            proj(t)
            return carry

        jax.lax.fori_loop(0, 3, qkv_body, 0)
        wo_copy.wait()
        for kc in range(NC):
            for h in range(H):
                tmp[kc, h * PAD:h * PAD + DH, :] = (
                    wo_raw[h * DH:(h + 1) * DH, kc * 128:(kc + 1) * 128].astype(F32))
        permute_from_tmp(wo_p)

        def attn_body(i, carry):
            r0 = pl.multiple_of(i * (4 * RC), 4 * RC)
            for j in range(4):
                attn_rows(r0 + j * RC, True)
            return carry

        jax.lax.fori_loop(0, NRC // 4, attn_body, 0)

    @pl.when(jnp.logical_and(s > 0, s < 2 * NB))
    def _front():
        ln1(False)
        out_proj()
        qkv_s[1:3, :, 0:HALO, :] = qkv_s[1:3, :, TM:TM + HALO, :]
        proj(0)
        ln2()
        proj(1)
        proj(2)

    @pl.when(s == 2 * NB)
    def _front_last():
        out_proj()
        ln2()

    @pl.when(s == 1)
    def _wait_mlp_weights():
        w1_copy.wait()
        w2_copy.wait()

    @pl.when(s > 0)
    def _back():
        mlp_attn()


def _build(TM=256, FC=512, RC=8, TOK=False):
    NB = S // TM
    any_spec = pl.BlockSpec(memory_space=pl.ANY)
    return pl.pallas_call(
        functools.partial(_kernel, TM=TM, FC=FC, RC=RC, TOK=TOK),
        grid=(2 * NB + 1,),
        in_specs=[
            pl.BlockSpec((TM, D), lambda s: (jnp.minimum(s, NB - 1), 0)),
            any_spec, any_spec, any_spec,
            pl.BlockSpec((1, F), lambda s: (0, 0)),
            any_spec,
            pl.BlockSpec((1, D), lambda s: (0, 0)),
        ],
        out_specs=pl.BlockSpec((TM, D), lambda s: (jnp.maximum(s - 1 - NB, 0), 0)),
        out_shape=jax.ShapeDtypeStruct((S, D), BF16),
        scratch_shapes=[
            pltpu.VMEM((3, D, D), BF16),
            pltpu.VMEM((D, D), BF16),
            pltpu.VMEM((3, D, D), BF16),
            pltpu.VMEM((D, D), BF16),
            pltpu.VMEM((D, F), BF16),
            pltpu.VMEM((F, D), BF16),
            pltpu.VMEM((NC, H * PAD, 128), F32),
            pltpu.VMEM((S, D), F32),
            pltpu.VMEM((TM, D), F32),
            pltpu.VMEM((TM, D), BF16),
            pltpu.VMEM((TM, D), BF16),
            pltpu.VMEM((3, NC, TM + HALO, 128), F32),
            pltpu.VMEM((TM, D), BF16),
            pltpu.SemaphoreType.DMA((6,)),
        ],
        compiler_params=pltpu.CompilerParams(
            dimension_semantics=("arbitrary",), vmem_limit_bytes=100 * 1024 * 1024),
    )


def _call(fn, A_x, A_wqkv, A_wo, B_x, B_w1, B_b1, B_w2, B_b2):
    del B_x
    out = fn(A_x.reshape(S, D), A_wqkv, A_wo, B_w1, B_b1.reshape(1, F), B_w2,
             B_b2.reshape(1, D))
    return out.reshape(1, S, D)


@jax.jit
def pallas_interleave_layers__sliding_local_dilated__dense_activation_gelu__prompt_kernel(
    A_x: jax.Array,
    A_wqkv: jax.Array,
    A_wo: jax.Array,
    B_x: jax.Array,
    B_w1: jax.Array,
    B_b1: jax.Array,
    B_w2: jax.Array,
    B_b2: jax.Array,
):
    return _call(_build(), A_x, A_wqkv, A_wo, B_x, B_w1, B_b1, B_w2, B_b2)
```

```python
import functools

import jax
import jax.numpy as jnp
import jax.experimental.pallas as pl
import jax.experimental.pallas.tpu as pltpu

S, D, F = 2048, 1024, 3584
H, DH, WIN, DIL = 32, 32, 8, 2
NC = D // 128
HALO = 16
EPS = 1e-5
SCALE = DH ** -0.5
LOG2E = 1.4426950408889634
PAD = DH + 1
F32, BF16 = jnp.float32, jnp.bfloat16
NT = (((1,), (1,)), ((), ()))


def _gelu(x):
    c = 0.7978845608028654
    t = jnp.tanh(x * (c + (c * 0.044715) * (x * x)))
    hx = 0.5 * x
    return hx + hx * t


def _kernel(x_ref, xp_ref, wqkv_hbm, wo_hbm, w1_hbm, b1_ref, w2_hbm, b2_ref, o_ref,
            wq_raw, wo_raw, wt, wo_p, w1, w2, tmp, xs, x1_s, xn_s, y_s, qkv_s, o_s, sems,
            *, TM, FC, RC, TOK, STEP, L1STEP, L1LAG, L2STEP, L2LAG):
    NB = S // TM
    s = pl.program_id(0)
    NFC = F // FC
    NRC = TM // RC
    row0 = pl.multiple_of((s % NB) * TM, TM)
    prow = pl.multiple_of(((s + NB - 1) % NB) * TM, TM)
    live = (jax.lax.broadcasted_iota(jnp.int32, (RC, 128), 0) + s) >= 0

    def tokens(r, step=1, n=256):
        return [r[(j % NRC) * RC:(j % NRC + 1) * RC, (j // NRC) * 128:(j // NRC + 1) * 128]
                for j in range(0, n, step)]

    def ln_rows(x, dst, r0, toks):
        m = jnp.sum(gate(tree(x), toks[0]), axis=1, keepdims=True) * (1.0 / D)
        x = [t - m for t in x]
        v = jnp.sum(gate(tree([t * t for t in x]), toks[1]), axis=1, keepdims=True) * (1.0 / D)
        r = gate(jnp.broadcast_to(jax.lax.rsqrt(v + EPS), (RC, 128)), toks[2])
        for c in range(NC):
            dst[r0:r0 + RC, c * 128:(c + 1) * 128] = (x[c] * r).astype(BF16)

    def ln_all(load, dst, toks, lag):
        for g in range(NRC):
            tk = [None] * 3 if toks is None else [toks[3 * (g + k * lag) + k] for k in range(3)]
            ln_rows([load(g * RC, c) for c in range(NC)], dst, g * RC, tk)

    def resid(ref, first, base):
        def load(r0, c):
            xin = ref[r0:r0 + RC, c * 128:(c + 1) * 128].astype(F32)
            if first is True:
                return xin
            return jnp.where(first, xin, xs[pl.ds(base + r0, RC), c * 128:(c + 1) * 128])
        return load

    def proj(t):
        r = jax.lax.dot_general(xn_s[...], wt[t], NT, preferred_element_type=F32)
        for c in range(NC):
            qkv_s[t, c, HALO:HALO + TM, :] = r[:, c * 128:(c + 1) * 128]
        return r

    def tree(p):
        return ((p[0] + p[1]) + (p[2] + p[3])) + ((p[4] + p[5]) + (p[6] + p[7]))

    def gate(x, tok):
        return x if tok is None else jnp.where(live, x, tok)

    def attn_qk(r0, toks=None):
        if TOK == 1 and toks is not None:
            lg = None
            for c in range(NC):
                q = gate(qkv_s[0, c, pl.ds(r0 + HALO, RC), :], toks[c])
                p = [q * qkv_s[1, c, pl.ds(r0 + HALO - DIL * w, RC), :] for w in range(WIN)]
                lg = p if lg is None else [a + b for a, b in zip(lg, p)]
            return lg
        q = [qkv_s[0, c, pl.ds(r0 + HALO, RC), :] for c in range(NC)]
        return [gate(tree([q[c] * qkv_s[1, c, pl.ds(r0 + HALO - DIL * w, RC), :] for c in range(NC)]),
                     None if toks is None else toks[w])
                for w in range(WIN)]

    def attn_softmax(lg, r0, masked):
        out = []
        for w, t in enumerate(lg):
            t = t + pltpu.roll(t, 64, 1)
            t = t + pltpu.roll(t, 32, 1)
            if w > 0 and masked:
                pos = row0 + r0 + jax.lax.broadcasted_iota(jnp.int32, (RC, 128), 0)
                t = jnp.where(pos >= DIL * w, t, -1e9 / SCALE)
            out.append(t)
        lg = out
        m = jnp.maximum(jnp.maximum(jnp.maximum(lg[0], lg[1]), jnp.maximum(lg[2], lg[3])),
                        jnp.maximum(jnp.maximum(lg[4], lg[5]), jnp.maximum(lg[6], lg[7])))
        e = [jnp.exp2((t - m) * (SCALE * LOG2E)) for t in lg]
        den = tree(e)
        inv = pl.reciprocal(den, approx=True)
        inv = inv * (2.0 - den * inv)
        return e, inv

    def attn_pv(e, inv, r0, toks=None):
        if TOK == 1 and toks is not None:
            o = None
            for w in range(WIN):
                ew = gate(e[w], toks[w])
                p = [ew * qkv_s[2, c, pl.ds(r0 + HALO - DIL * w, RC), :] for c in range(NC)]
                o = p if o is None else [a + b for a, b in zip(o, p)]
            for c in range(NC):
                o_s[pl.ds(r0, RC), c * 128:(c + 1) * 128] = (o[c] * inv).astype(BF16)
            return
        for c in range(NC):
            t = tree([e[w] * qkv_s[2, c, pl.ds(r0 + HALO - DIL * w, RC), :] for w in range(WIN)])
            t = t * gate(inv, None if toks is None else toks[c])
            o_s[pl.ds(r0, RC), c * 128:(c + 1) * 128] = t.astype(BF16)

    def attn_rows(r0, masked):
        e, inv = attn_softmax(attn_qk(r0), r0, masked)
        attn_pv(e, inv, r0)

    def out_proj():
        res = jnp.where(s <= NB, xp_ref[...].astype(F32), xs[pl.ds(prow, TM), :])
        x1 = res + jnp.dot(o_s[...], wo_p[...], preferred_element_type=F32)
        x1_s[...] = x1
        return x1

    def ln2(toks, lag):
        ln_all(lambda r0, c: x1_s[r0:r0 + RC, c * 128:(c + 1) * 128], y_s, toks, lag)

    def mlp_attn():
        g = 0
        toks = []
        for c in range(NFC):
            h = jnp.dot(y_s[...], w1[:, c * FC:(c + 1) * FC], preferred_element_type=F32)
            h = _gelu(h + b1_ref[:, c * FC:(c + 1) * FC].astype(F32)).astype(BF16)
            acc = x1_s[...] + jnp.dot(h, w2[c * FC:(c + 1) * FC, :], preferred_element_type=F32)
            if c < NFC - 1:
                x1_s[...] = acc
            else:
                acc = acc + b2_ref[...].astype(F32)
                xs[pl.ds(prow, TM), :] = acc
                o_ref[...] = acc.astype(BF16)
            if not TOK:
                n = min(NRC - g, -(-NRC // (NFC - 1)))
                for j in range(n):
                    attn_rows(g * RC, g * RC < HALO)
                    g += 1
                continue
            toks += tokens(acc, STEP)
            while g <= NRC and len(toks) >= 16:
                if g < NRC:
                    lg = attn_qk(g * RC, toks[:8])
                if g > 0:
                    attn_pv(*sm, (g - 1) * RC, toks[8:16])
                if g < NRC:
                    sm = attn_softmax(lg, g * RC, g * RC < HALO)
                toks = toks[16:]
                g += 1
        assert not TOK or g == NRC + 1

    def wq_copy(t):
        return pltpu.make_async_copy(wqkv_hbm.at[:, pl.ds(t * D, D)], wq_raw.at[t], sems.at[t])

    wo_copy = pltpu.make_async_copy(wo_hbm, wo_raw, sems.at[3])
    w1_copy = pltpu.make_async_copy(w1_hbm, w1, sems.at[4])
    w2_copy = pltpu.make_async_copy(w2_hbm, w2, sems.at[5])

    def permute_from_tmp(dst):
        for d in range(DH):
            for kc in range(NC):
                dst[d * H:(d + 1) * H, kc * 128:(kc + 1) * 128] = (
                    tmp[kc, pl.ds(d, H, stride=PAD), :].astype(BF16))

    @pl.when(s == 0)
    def _prologue():
        for t in range(3):
            wq_copy(t).start()
        wo_copy.start()
        w1_copy.start()
        w2_copy.start()
        ln_all(resid(x_ref, True, 0), xn_s, None, 0)
        qkv_s[:, :, 0:HALO, :] = jnp.zeros((3, NC, HALO, 128), F32)
        o_ref[...] = jnp.zeros(o_ref.shape, BF16)
        eye = (jax.lax.broadcasted_iota(jnp.int32, (128, 128), 0)
               == jax.lax.broadcasted_iota(jnp.int32, (128, 128), 1)).astype(BF16)

        def qkv_body(t, carry):
            wq_copy(t).wait()
            for c in range(NC):
                tile = jax.lax.dot_general(eye, wq_raw[t, :, c * 128:(c + 1) * 128], NT,
                                           preferred_element_type=F32)
                for kc in range(NC):
                    for hh in range(4):
                        tmp[kc, (4 * c + hh) * PAD:(4 * c + hh) * PAD + DH, :] = (
                            tile[hh * DH:(hh + 1) * DH, kc * 128:(kc + 1) * 128])
            permute_from_tmp(wt.at[t])
            proj(t)
            return carry

        jax.lax.fori_loop(0, 3, qkv_body, 0)
        wo_copy.wait()
        for kc in range(NC):
            for h in range(H):
                tmp[kc, h * PAD:h * PAD + DH, :] = (
                    wo_raw[h * DH:(h + 1) * DH, kc * 128:(kc + 1) * 128].astype(F32))
        permute_from_tmp(wo_p)

        def attn_body(i, carry):
            r0 = pl.multiple_of(i * (4 * RC), 4 * RC)
            for j in range(4):
                attn_rows(r0 + j * RC, True)
            return carry

        jax.lax.fori_loop(0, NRC // 4, attn_body, 0)

    @pl.when(jnp.logical_and(s > 0, s < 2 * NB))
    def _front():
        x1 = out_proj()
        ln_all(resid(x_ref, s < NB, row0), xn_s, tokens(x1, L1STEP), L1LAG)
        qkv_s[1:3, :, 0:HALO, :] = qkv_s[1:3, :, TM:TM + HALO, :]
        toks = tokens(proj(0), L2STEP) + tokens(proj(1), L2STEP) + tokens(proj(2), L2STEP)
        ln2(toks, L2LAG)

    @pl.when(s == 2 * NB)
    def _front_last():
        out_proj()
        ln2(None, 0)

    @pl.when(s == 1)
    def _wait_mlp_weights():
        w1_copy.wait()
        w2_copy.wait()

    @pl.when(s > 0)
    def _back():
        mlp_attn()


def _build(TM=256, FC=512, RC=8, TOK=2, STEP=3, L1STEP=2, L1LAG=2, L2STEP=6, L2LAG=1):
    NB = S // TM
    any_spec = pl.BlockSpec(memory_space=pl.ANY)
    return pl.pallas_call(
        functools.partial(_kernel, TM=TM, FC=FC, RC=RC, TOK=TOK, STEP=STEP,
                          L1STEP=L1STEP, L1LAG=L1LAG, L2STEP=L2STEP, L2LAG=L2LAG),
        grid=(2 * NB + 1,),
        in_specs=[
            pl.BlockSpec((TM, D), lambda s: (jnp.minimum(s, NB - 1), 0)),
            pl.BlockSpec((TM, D), lambda s: (jnp.clip(s - 1, 0, NB - 1), 0)),
            any_spec, any_spec, any_spec,
            pl.BlockSpec((1, F), lambda s: (0, 0)),
            any_spec,
            pl.BlockSpec((1, D), lambda s: (0, 0)),
        ],
        out_specs=pl.BlockSpec((TM, D), lambda s: (jnp.maximum(s - 1 - NB, 0), 0)),
        out_shape=jax.ShapeDtypeStruct((S, D), BF16),
        scratch_shapes=[
            pltpu.VMEM((3, D, D), BF16),
            pltpu.VMEM((D, D), BF16),
            pltpu.VMEM((3, D, D), BF16),
            pltpu.VMEM((D, D), BF16),
            pltpu.VMEM((D, F), BF16),
            pltpu.VMEM((F, D), BF16),
            pltpu.VMEM((NC, H * PAD, 128), F32),
            pltpu.VMEM((S, D), F32),
            pltpu.VMEM((TM, D), F32),
            pltpu.VMEM((TM, D), BF16),
            pltpu.VMEM((TM, D), BF16),
            pltpu.VMEM((3, NC, TM + HALO, 128), F32),
            pltpu.VMEM((TM, D), BF16),
            pltpu.SemaphoreType.DMA((6,)),
        ],
        compiler_params=pltpu.CompilerParams(
            dimension_semantics=("arbitrary",), vmem_limit_bytes=100 * 1024 * 1024),
    )


def _call(fn, A_x, A_wqkv, A_wo, B_x, B_w1, B_b1, B_w2, B_b2):
    del B_x
    x = A_x.reshape(S, D)
    out = fn(x, x, A_wqkv, A_wo, B_w1, B_b1.reshape(1, F), B_w2,
             B_b2.reshape(1, D))
    return out.reshape(1, S, D)


@jax.jit
def pallas_interleave_layers__sliding_local_dilated__dense_activation_gelu__prompt_kernel(
    A_x: jax.Array,
    A_wqkv: jax.Array,
    A_wo: jax.Array,
    B_x: jax.Array,
    B_w1: jax.Array,
    B_b1: jax.Array,
    B_w2: jax.Array,
    B_b2: jax.Array,
):
    return _call(_build(), A_x, A_wqkv, A_wo, B_x, B_w1, B_b1, B_w2, B_b2)
```

```python
import functools

import jax
import jax.numpy as jnp
import jax.experimental.pallas as pl
import jax.experimental.pallas.tpu as pltpu

S, D, F = 2048, 1024, 3584
H, DH, WIN, DIL = 32, 32, 8, 2
NC = D // 128
HALO = 16
EPS = 1e-5
SCALE = DH ** -0.5
LOG2E = 1.4426950408889634
PAD = DH + 1
F32, BF16, U32 = jnp.float32, jnp.bfloat16, jnp.uint32
TM, RC = 256, 8
HM, NB, NRC, NF2 = TM // 2, S // TM, TM // RC, F // 256
NN = (((1,), (0,)), ((), ()))
NT = (((1,), (1,)), ((), ()))


def _gelu(x):
    c = 0.7978845608028654
    t = jnp.tanh(x * (c + (c * 0.044715) * (x * x)))
    hx = 0.5 * x
    return hx + hx * t


def _tree(p):
    return ((p[0] + p[1]) + (p[2] + p[3])) + ((p[4] + p[5]) + (p[6] + p[7]))


def _pack(x):
    return pltpu.bitcast(x.astype(BF16), U32)


def _unpack(x):
    return pltpu.bitcast(x, BF16)


def _lhs_ops(a11, a12, a21, a22):
    return [a11 + a22, a21 + a22, a11, a22, a11 + a12, a21 - a11, a12 - a22]


def _rhs_ops(b11, b12, b21, b22):
    return [b11 + b22, b11, b12 - b22, b21 - b11, b22, b11 + b12, b21 + b22]


def _strassen(prod):
    m1 = prod(0)
    m4 = prod(3)
    c11 = m1 + m4
    m2 = prod(1)
    c21 = m2 + m4
    c22 = m1 - m2
    c11 = c11 + prod(6)
    m5 = prod(4)
    c11 = c11 - m5
    m3 = prod(2)
    c12 = m3 + m5
    c22 = (c22 + m3) + prod(5)
    return c11, c12, c21, c22


def _kernel(x_ref, xp_ref, wqkv_hbm, wo_hbm, w1_hbm, b1_ref, w2_hbm, b2_ref, o_ref,
            wq_raw, wo_raw, w1_raw, w2_raw, bq, bo, bw1, bw2, tmp, xs, x1_s, st1, st2,
            a_x, a_y, a_o, a_h, qkv_s, sems, *, P):
    s = pl.program_id(0)
    row0 = pl.multiple_of((s % NB) * TM, TM)
    prow = pl.multiple_of(((s + NB - 1) % NB) * TM, TM)
    live = (jax.lax.broadcasted_iota(jnp.int32, (RC, 128), 0) + s) >= 0
    order = [g for j in range(NRC // 4) for g in (2 * j, 2 * j + 1, NRC // 2 + 2 * j, NRC // 2 + 2 * j + 1)]
    cs = lambda c: slice(c * 128, (c + 1) * 128)

    def gate(x, tok):
        return x if tok is None else jnp.where(live, x, tok)

    def lhs(buf, i, k0=0, k1=4):
        return jnp.concatenate([_unpack(buf[i, k]) for k in range(k0, k1)], axis=1)

    def dot(a, b, toks, dims=NN):
        r = jax.lax.dot_general(a, b, dims, preferred_element_type=F32)
        toks.extend(r[j * RC:(j + 1) * RC, :] for j in range(HM // RC))
        return r

    def combine(src, dst, j, toks=None):
        r16 = j * 16 if isinstance(j, int) else pl.multiple_of(j * 16, 16)
        r8 = j * 8 if isinstance(j, int) else pl.multiple_of(j * 8, 8)
        for c in range(4):
            def ld(r, cc, tok=None):
                return jnp.concatenate([gate(src[pl.ds(r, RC), cs(cc)], tok),
                                        src[pl.ds(r + RC, RC), cs(cc)]], axis=0)
            tok = None if toks is None else toks[c]
            ops = _lhs_ops(ld(r16, c, tok), ld(r16, c + 4), ld(HM + r16, c), ld(HM + r16, c + 4, tok))
            for i in range(7):
                dst[i, c, pl.ds(r8, 8), :] = _pack(ops[i])

    def ln_rows(x, dst, r0, toks):
        m = jnp.sum(gate(_tree(x), toks[0]), axis=1, keepdims=True) * (1.0 / D)
        x = [t - m for t in x]
        v = jnp.sum(gate(_tree([t * t for t in x]), toks[1]), axis=1, keepdims=True) * (1.0 / D)
        r = gate(jnp.broadcast_to(jax.lax.rsqrt(v + EPS), (RC, 128)), toks[2])
        for c in range(NC):
            dst[r0:r0 + RC, cs(c)] = x[c] * r

    def ln_all(load, stage, dst, toks=None, lag=0):
        for n, g in enumerate(order):
            tk = [None] * 3 if toks is None else [toks[4 * (n + k * lag) + k] for k in range(3)]
            ln_rows([load(g * RC, c) for c in range(NC)], stage, g * RC, tk)
            if n % 4 == 3:
                combine(stage, dst, n // 4,
                        None if toks is None else [toks[4 * (n + 1 + c + 2 * lag) + 3] for c in range(4)])

    def resid(ref, first, base):
        def load(r0, c, rows=RC):
            xin = ref[r0:r0 + rows, cs(c)].astype(F32)
            if first is True:
                return xin
            return jnp.where(first, xin, xs[pl.ds(base + r0, rows), cs(c)])
        return load

    def proj(t, av, toks):
        for a in range(4):
            c = _strassen(lambda i: dot(av[i], lhs(bq.at[t, a], i), toks, NT))
            for k in range(4):
                r = HALO + (k // 2) * HM
                qkv_s[t, a + 4 * (k % 2), r:r + HM, :] = c[k]

    def attn_qk(r0, toks=None):
        q = [qkv_s[0, c, pl.ds(r0 + HALO, RC), :] for c in range(NC)]
        return [gate(_tree([q[c] * qkv_s[1, c, pl.ds(r0 + HALO - DIL * w, RC), :] for c in range(NC)]),
                     None if toks is None else toks[w])
                for w in range(WIN)]

    def attn_softmax(lg, r0, masked):
        out = []
        for w, t in enumerate(lg):
            t = t + pltpu.roll(t, 64, 1)
            t = t + pltpu.roll(t, 32, 1)
            if w > 0 and masked:
                pos = row0 + r0 + jax.lax.broadcasted_iota(jnp.int32, (RC, 128), 0)
                t = jnp.where(pos >= DIL * w, t, -1e9 / SCALE)
            out.append(t)
        lg = out
        m = jnp.maximum(jnp.maximum(jnp.maximum(lg[0], lg[1]), jnp.maximum(lg[2], lg[3])),
                        jnp.maximum(jnp.maximum(lg[4], lg[5]), jnp.maximum(lg[6], lg[7])))
        e = [jnp.exp2((t - m) * (SCALE * LOG2E)) for t in lg]
        den = _tree(e)
        inv = pl.reciprocal(den, approx=True)
        inv = inv * (2.0 - den * inv)
        return e, inv

    def attn_pv(e, inv, r0, toks=None):
        for c in range(NC):
            t = _tree([e[w] * qkv_s[2, c, pl.ds(r0 + HALO - DIL * w, RC), :] for w in range(WIN)])
            st1[pl.ds(r0, RC), cs(c)] = t * gate(inv, None if toks is None else toks[c])

    def attn_paced(toks):
        sm = None
        for n in range(NRC + 2):
            tk = toks[17 * n:17 * (n + 1)]
            if n < NRC:
                lg = attn_qk(order[n] * RC, tk[:8])
            if 0 < n <= NRC:
                attn_pv(*sm, order[n - 1] * RC, tk[8:16])
            if n < NRC:
                sm = attn_softmax(lg, order[n] * RC, order[n] * RC < HALO)
            if n > 1 and n % 4 == 1:
                combine(st1, a_o, n // 4 - 1, [tk[3], tk[7], tk[11], tk[16]])

    def out_proj(toks):
        av = [lhs(a_o, i) for i in range(7)]
        res = resid(xp_ref, s <= NB, prow)
        for a in range(4):
            c = _strassen(lambda i: dot(av[i], _unpack(bo[a, i]), toks))
            for k in range(4):
                r, cc = (k // 2) * HM, a + 4 * (k % 2)
                x1_s[r:r + HM, cs(cc)] = res(r, cc, HM) + c[k]

    def ln2(toks=None, lag=0):
        ln_all(lambda r0, c: x1_s[r0:r0 + RC, cs(c)], st2, a_y, toks, lag)

    def mlp_attn():
        t1, t2 = [], []
        av = [lhs(a_y, i) for i in range(7)]
        for j in range(NF2):
            c = _strassen(lambda i: dot(av[i], _unpack(bw1[j, i]), t1))
            bl = b1_ref[:, cs(j)].astype(F32)
            br = b1_ref[:, cs(j + NF2)].astype(F32)
            ops = _lhs_ops(_gelu(c[0] + bl), _gelu(c[1] + br), _gelu(c[2] + bl), _gelu(c[3] + br))
            for i in range(7):
                a_h[i, j] = _pack(ops[i])

        def prod2(a, i):
            acc = None
            for k0 in range(0, NF2, 4):
                k1 = min(k0 + 4, NF2)
                r = dot(lhs(a_h, i, k0, k1), _unpack(bw2[a, i, k0 * 64:k1 * 64, :]), t2)
                acc = r if acc is None else acc + r
            return acc

        for a in range(4):
            c = _strassen(functools.partial(prod2, a))
            for k in range(4):
                r, cc = (k // 2) * HM, a + 4 * (k % 2)
                y = (x1_s[r:r + HM, cs(cc)] + b2_ref[:, cs(cc)].astype(F32)) + c[k]
                xs[pl.ds(prow + r, HM), cs(cc)] = y
                o_ref[r:r + HM, cs(cc)] = y.astype(BF16)
        attn_paced((t1[P["a0"]::P["a1"]] + t2[::P["a2"]]))

    def wq_copy(t):
        return pltpu.make_async_copy(wqkv_hbm.at[:, pl.ds(t * D, D)], wq_raw.at[t], sems.at[t])

    wo_copy = pltpu.make_async_copy(wo_hbm, wo_raw, sems.at[3])
    w1_copy = pltpu.make_async_copy(w1_hbm, w1_raw, sems.at[4])
    w2_copy = pltpu.make_async_copy(w2_hbm, w2_raw, sems.at[5])

    def perm(k, d):
        return tmp[k, pl.ds(d, H, stride=PAD), :]

    @pl.when(s == 0)
    def _prologue():
        for t in range(3):
            wq_copy(t).start()
        wo_copy.start()
        w1_copy.start()
        w2_copy.start()
        ln_all(resid(x_ref, True, 0), st1, a_x)
        qkv_s[:, :, 0:HALO, :] = jnp.zeros((3, NC, HALO, 128), F32)
        o_ref[...] = jnp.zeros(o_ref.shape, BF16)
        eye = (jax.lax.broadcasted_iota(jnp.int32, (128, 128), 0)
               == jax.lax.broadcasted_iota(jnp.int32, (128, 128), 1)).astype(BF16)

        def qkv_body(t, carry):
            wq_copy(t).wait()
            for c in range(NC):
                tile = jax.lax.dot_general(eye, wq_raw[t, :, cs(c)], NT, preferred_element_type=F32)
                for k in range(NC):
                    for hh in range(4):
                        tmp[k, (4 * c + hh) * PAD:(4 * c + hh) * PAD + DH, :] = (
                            tile[hh * DH:(hh + 1) * DH, cs(k)])
            for d in range(DH // 2):
                for k in range(4):
                    ops = _rhs_ops(perm(k, d), perm(k, d + 16), perm(k + 4, d), perm(k + 4, d + 16))
                    for i in range(7):
                        bq[t, d // 4, i, k, (d % 4) * 16:(d % 4 + 1) * 16, :] = _pack(ops[i])
            proj(t, [lhs(a_x, i) for i in range(7)], [])
            return carry

        jax.lax.fori_loop(0, 3, qkv_body, 0)
        wo_copy.wait()
        for c in range(NC):
            for h in range(H):
                tmp[c, h * PAD:h * PAD + DH, :] = wo_raw[h * DH:(h + 1) * DH, cs(c)].astype(F32)
        for d in range(DH // 2):
            for c in range(4):
                ops = _rhs_ops(perm(c, d), perm(c + 4, d), perm(c, d + 16), perm(c + 4, d + 16))
                for i in range(7):
                    bo[c, i, d * 16:(d + 1) * 16, :] = _pack(ops[i])

        def attn_body(j, carry):
            r16 = pl.multiple_of(j * 16, 16)
            for r0 in (r16, r16 + RC, HM + r16, HM + r16 + RC):
                e, inv = attn_softmax(attn_qk(r0), r0, True)
                attn_pv(e, inv, r0)
            combine(st1, a_o, j)
            return carry

        jax.lax.fori_loop(0, NRC // 4, attn_body, 0)

    @pl.when(jnp.logical_and(s > 0, s < 2 * NB))
    def _front():
        toks = []
        out_proj(toks)
        ln_all(resid(x_ref, s < NB, row0), st1, a_x, toks[::P["l1"]], P["l1lag"])
        qkv_s[1:3, :, 0:HALO, :] = qkv_s[1:3, :, TM:TM + HALO, :]
        toks = []
        av = [lhs(a_x, i) for i in range(7)]
        for t in range(3):
            proj(t, av, toks)
        ln2(toks[P["l20"]::P["l2"]], P["l2lag"])

    @pl.when(s == 2 * NB)
    def _front_last():
        out_proj([])
        ln2()

    @pl.when(s == 1)
    def _mlp_weights():
        w1_copy.wait()

        def w1_body(n, carry):
            r = pl.multiple_of(n * 32, 32)
            ld = lambda r_, j: w1_raw[pl.ds(r_, 32), cs(j)].astype(F32)
            for j in range(NF2):
                ops = _rhs_ops(ld(r, j), ld(r, j + NF2), ld(D // 2 + r, j), ld(D // 2 + r, j + NF2))
                for i in range(7):
                    bw1[j, i, pl.ds(pl.multiple_of(n * 16, 16), 16), :] = _pack(ops[i])
            return carry

        jax.lax.fori_loop(0, D // 2 // 32, w1_body, 0)
        w2_copy.wait()

        def w2_body(n, carry):
            r = pl.multiple_of(n * 128, 128)
            ld = lambda r_, c: w2_raw[pl.ds(r_, 128), cs(c)].astype(F32)
            for c in range(4):
                ops = _rhs_ops(ld(r, c), ld(r, c + 4), ld(F // 2 + r, c), ld(F // 2 + r, c + 4))
                for i in range(7):
                    bw2[c, i, pl.ds(pl.multiple_of(n * 64, 64), 64), :] = _pack(ops[i])
            return carry

        jax.lax.fori_loop(0, NF2, w2_body, 0)

    @pl.when(s > 0)
    def _back():
        mlp_attn()


def _build(**kw):
    P = dict(a0=10 ** 6, a1=1, a2=3, l1=2, l1lag=4, l20=16, l2=8, l2lag=1)
    P.update(kw)
    any_spec = pl.BlockSpec(memory_space=pl.ANY)
    return pl.pallas_call(
        functools.partial(_kernel, P=P),
        grid=(2 * NB + 1,),
        in_specs=[
            pl.BlockSpec((TM, D), lambda s: (jnp.minimum(s, NB - 1), 0)),
            pl.BlockSpec((TM, D), lambda s: (jnp.clip(s - 1, 0, NB - 1), 0)),
            any_spec, any_spec, any_spec,
            pl.BlockSpec((1, F), lambda s: (0, 0)),
            any_spec,
            pl.BlockSpec((1, D), lambda s: (0, 0)),
        ],
        out_specs=pl.BlockSpec((TM, D), lambda s: (jnp.maximum(s - 1 - NB, 0), 0)),
        out_shape=jax.ShapeDtypeStruct((S, D), BF16),
        scratch_shapes=[
            pltpu.VMEM((3, D, D), BF16),
            pltpu.VMEM((D, D), BF16),
            pltpu.VMEM((D, F), BF16),
            pltpu.VMEM((F, D), BF16),
            pltpu.VMEM((3, 4, 7, 4, 64, 128), U32),
            pltpu.VMEM((4, 7, 256, 128), U32),
            pltpu.VMEM((NF2, 7, 256, 128), U32),
            pltpu.VMEM((4, 7, NF2 * 64, 128), U32),
            pltpu.VMEM((NC, H * PAD, 128), F32),
            pltpu.VMEM((S, D), F32),
            pltpu.VMEM((TM, D), F32),
            pltpu.VMEM((TM, D), F32),
            pltpu.VMEM((TM, D), F32),
            pltpu.VMEM((7, 4, 64, 128), U32),
            pltpu.VMEM((7, 4, 64, 128), U32),
            pltpu.VMEM((7, 4, 64, 128), U32),
            pltpu.VMEM((7, NF2, 64, 128), U32),
            pltpu.VMEM((3, NC, TM + HALO, 128), F32),
            pltpu.SemaphoreType.DMA((6,)),
        ],
        compiler_params=pltpu.CompilerParams(
            dimension_semantics=("arbitrary",), vmem_limit_bytes=110 * 1024 * 1024),
    )


def _call(fn, A_x, A_wqkv, A_wo, B_x, B_w1, B_b1, B_w2, B_b2):
    del B_x
    x = A_x.reshape(S, D)
    out = fn(x, x, A_wqkv, A_wo, B_w1, B_b1.reshape(1, F), B_w2,
             B_b2.reshape(1, D))
    return out.reshape(1, S, D)


@jax.jit
def pallas_interleave_layers__sliding_local_dilated__dense_activation_gelu__prompt_kernel(
    A_x: jax.Array,
    A_wqkv: jax.Array,
    A_wo: jax.Array,
    B_x: jax.Array,
    B_w1: jax.Array,
    B_b1: jax.Array,
    B_w2: jax.Array,
    B_b2: jax.Array,
):
    return _call(_build(), A_x, A_wqkv, A_wo, B_x, B_w1, B_b1, B_w2, B_b2)
```

```python
import functools

import jax
import jax.numpy as jnp
import jax.experimental.pallas as pl
import jax.experimental.pallas.tpu as pltpu

S, D, F = 2048, 1024, 3584
H, DH, WIN, DIL = 32, 32, 8, 2
NC = D // 128
HALO = 16
EPS = 1e-5
SCALE = DH ** -0.5
LOG2E = 1.4426950408889634
PAD = DH + 1
F32, BF16, U32 = jnp.float32, jnp.bfloat16, jnp.uint32
TM, RC = 256, 8
HM, QM, NB, NRC = TM // 2, TM // 4, S // TM, TM // RC
NF4 = F // 512
SORD = (0, 3, 1, 6, 4, 2, 5)
NN = (((1,), (0,)), ((), ()))
NT = (((1,), (1,)), ((), ()))


def _gelu(x):
    c = 0.7978845608028654
    t = jnp.tanh(x * (c + (c * 0.044715) * (x * x)))
    hx = 0.5 * x
    return hx + hx * t


def _tree(p):
    return ((p[0] + p[1]) + (p[2] + p[3])) + ((p[4] + p[5]) + (p[6] + p[7]))


def _lhs_ops(a11, a12, a21, a22):
    return [a11 + a22, a21 + a22, a11, a22, a11 + a12, a21 - a11, a12 - a22]


def _rhs_ops(b11, b12, b21, b22):
    return [b11 + b22, b11, b12 - b22, b21 - b11, b22, b11 + b12, b21 + b22]


def _ops2(ops, blk, gate=None):
    outer = [[ops(blk[r][c], blk[r][c + 2], blk[r + 2][c], blk[r + 2][c + 2]) for c in range(2)]
             for r in range(2)]
    g = (lambda i, x: x) if gate is None else gate
    return [o for i in range(7)
            for o in ops(g(i, outer[0][0][i]), outer[0][1][i], outer[1][0][i], g(i, outer[1][1][i]))]


def _bf(u):
    return pltpu.bitcast(u, BF16)


def _strassen(prod):
    m1 = prod(0)
    m4 = prod(3)
    c11 = m1 + m4
    m2 = prod(1)
    c21 = m2 + m4
    c22 = m1 - m2
    c11 = c11 + prod(6)
    m5 = prod(4)
    c11 = c11 - m5
    m3 = prod(2)
    c12 = m3 + m5
    c22 = (c22 + m3) + prod(5)
    return c11, c12, c21, c22


def _strassen2(prod):
    c = _strassen(lambda i: jnp.concatenate(_strassen(lambda k: prod(7 * i + k)), axis=0))
    n = c[0].shape[0] // 4
    return [[c[2 * (r // 2) + q // 2][(2 * (r % 2) + q % 2) * n:(2 * (r % 2) + q % 2 + 1) * n]
             for q in range(4)] for r in range(4)]


def _kernel(x_hbm, wqkv_hbm, wo_hbm, w1_hbm, b1_hbm, w2_hbm, b2_hbm, o_hbm,
            x_s, o_s, b1_raw, b2_raw, b1_s, b2_s,
            wq_raw, wo_raw, w1_raw, w2_raw, bq, bo, bw1, bw2, tmp, xs, x1_s, st1, st2,
            a_x, a_y, a_o, a_h, qkv_s, sems, *, P):
    s = pl.program_id(0)
    bq_u, bo_u, bw1_u, bw2_u, ax_u, ay_u, ao_u, ah_u = (
        r.bitcast(U32) for r in (bq, bo, bw1, bw2, a_x, a_y, a_o, a_h))
    row0 = pl.multiple_of((s % NB) * TM, TM)
    prow = pl.multiple_of(((s + NB - 1) % NB) * TM, TM)
    live = (jax.lax.broadcasted_iota(jnp.int32, (RC, 128), 0) + s) >= 0
    order = [g for j in range(NRC // 4) for g in (2 * j, 2 * j + 1, NRC // 2 + 2 * j, NRC // 2 + 2 * j + 1)]
    order2 = [8 * q + 2 * g + n for g in range(4) for q in range(4) for n in range(2)]
    cs = lambda c: slice(c * 128, (c + 1) * 128)

    def gate(x, tok):
        return x if tok is None else jnp.where(live, x, tok)

    def gate16(x, tok, tok2=None):
        return jnp.concatenate([gate(x[:RC], tok), gate(x[RC:], tok2)], axis=0)

    def lhs(buf, i, k0=0, k1=4):
        return jnp.concatenate([_bf(buf[i, k]) for k in range(k0, k1)], axis=1)

    def dot(a, b, toks, dims=NN):
        r = jax.lax.dot_general(a, b, dims, preferred_element_type=F32)
        toks.extend(r[j * RC:(j + 1) * RC, :] for j in range(r.shape[0] // RC))
        return r

    def combine(src, dst, j, toks=None):
        r16 = j * 16 if isinstance(j, int) else pl.multiple_of(j * 16, 16)
        for c in range(4):
            tok = None if toks is None else toks[c]
            ld = lambda r, cc: src[cc, pl.ds(r + r16, 16), :]
            ops = _lhs_ops(gate16(ld(0, c), tok), ld(0, c + 4), ld(HM, c), gate16(ld(HM, c + 4), tok))
            for i in range(7):
                dst[i, c, pl.ds(r16, 16), :] = ops[i].astype(BF16)

    def combine2(g, kk, toks=None):
        ops = _ops2(_lhs_ops, [[st2[2 * q + kk, QM * r + 16 * g:QM * r + 16 * g + 16, :]
                                for q in range(4)] for r in range(4)],
                    None if toks is None else lambda i, x: gate16(x, toks[i]))
        for p in range(49):
            a_y[p, kk, 16 * g:16 * g + 16, :] = ops[p].astype(BF16)

    def ln_rows(x, dst, r0, toks, chain, dep):
        prev = chain[-dep] if toks[0] is not None and len(chain) >= dep else None
        m = jnp.sum(gate(gate(_tree(x), toks[0]), prev), axis=1, keepdims=True) * (1.0 / D)
        x = [t - m for t in x]
        v = jnp.sum(gate(_tree([t * t for t in x]), toks[1]), axis=1, keepdims=True) * (1.0 / D)
        chain.append(jnp.broadcast_to(jax.lax.rsqrt(v + EPS), (RC, 128)))
        r = gate(chain[-1], toks[2])
        for c in range(NC):
            dst[c, r0:r0 + RC, :] = x[c] * r

    def ln_all(load, stage, dst, toks=None, lag=0):
        chain = []
        for n, g in enumerate(order):
            tk = [None] * 3 if toks is None else [toks[4 * (n + k * lag) + k] for k in range(3)]
            ln_rows([load(g * RC, c) for c in range(NC)], stage, g * RC, tk, chain, P["l1dep"])
            if n % 4 == 3:
                combine(stage, dst, n // 4,
                        None if toks is None else [toks[4 * (n + 1 + c + 2 * lag) + 3] for c in range(4)])

    def resid(first, base):
        def load(r0, c, rows=RC):
            xin = x_s[pl.ds(base + r0, rows), cs(c)].astype(F32)
            if first is True:
                return xin
            return jnp.where(first, xin, xs[pl.ds(base + r0, rows), cs(c)])
        return load

    def proj(t, av, toks, cols=range(4)):
        for a in cols:
            c = _strassen(lambda i: dot(av[i], jnp.concatenate([_bf(bq_u[t, a, i, k]) for k in range(4)], axis=1), toks, NT))
            for k in range(4):
                r = HALO + (k // 2) * HM
                qkv_s[t, a + 4 * (k % 2), r:r + HM, :] = c[k]

    def attn_qk(r0, toks=None):
        q = [qkv_s[0, c, pl.ds(r0 + HALO, RC), :] for c in range(NC)]
        return [gate(_tree([q[c] * qkv_s[1, c, pl.ds(r0 + HALO - DIL * w, RC), :] for c in range(NC)]),
                     None if toks is None else toks[w])
                for w in range(WIN)]

    def attn_softmax(lg, r0, masked):
        out = []
        for w, t in enumerate(lg):
            t = t + pltpu.roll(t, 64, 1)
            t = t + pltpu.roll(t, 32, 1)
            if w > 0 and masked:
                pos = row0 + r0 + jax.lax.broadcasted_iota(jnp.int32, (RC, 128), 0)
                t = jnp.where(pos >= DIL * w, t, -1e9 / SCALE)
            out.append(t)
        lg = out
        m = jnp.maximum(jnp.maximum(jnp.maximum(lg[0], lg[1]), jnp.maximum(lg[2], lg[3])),
                        jnp.maximum(jnp.maximum(lg[4], lg[5]), jnp.maximum(lg[6], lg[7])))
        e = [jnp.exp2((t - m) * (SCALE * LOG2E)) for t in lg]
        den = _tree(e)
        inv = pl.reciprocal(den, approx=True)
        inv = inv * (2.0 - den * inv)
        return e, inv

    def attn_pv(e, inv, r0, toks=None):
        for c in range(NC):
            t = _tree([e[w] * qkv_s[2, c, pl.ds(r0 + HALO - DIL * w, RC), :] for w in range(WIN)])
            st1[c, pl.ds(r0, RC), :] = t * gate(inv, None if toks is None else toks[c])

    def attn_paced(toks):
        sm = None
        for n in range(NRC + 2):
            tk = toks[17 * n:17 * (n + 1)]
            if n < NRC:
                lg = attn_qk(order[n] * RC, tk[:8])
            if 0 < n <= NRC:
                attn_pv(*sm, order[n - 1] * RC, tk[8:16])
            if n < NRC:
                sm = attn_softmax(lg, order[n] * RC, order[n] * RC < HALO)
            if n > 1 and n % 4 == 1:
                combine(st1, a_o, n // 4 - 1, [tk[3], tk[7], tk[11], tk[16]])

    def out_proj(toks):
        av = [lhs(ao_u, i) for i in range(7)]
        res = resid(s <= NB, prow)
        for a in range(4):
            c = _strassen(lambda i: dot(av[i], _bf(bo_u[a, i]), toks))
            for k in range(4):
                r, cc = (k // 2) * HM, a + 4 * (k % 2)
                x1_s[r:r + HM, cs(cc)] = res(r, cc, HM) + c[k]

    def ln2(toks=None, lag=0):
        chain = []
        for n, g in enumerate(order2):
            tk = [None] * 3 if toks is None else [toks[4 * (n + k * lag) + k] for k in range(3)]
            ln_rows([x1_s[g * RC:(g + 1) * RC, cs(c)] for c in range(NC)], st2, g * RC, tk, chain, P["l2dep"])
            if n % 8 == 7:
                for kk in range(2):
                    n0 = 4 * (n + 2 * lag + 1) + P["l2c"] * 7 * kk + 1
                    combine2(n // 8, kk, None if toks is None else toks[n0::P["l2c"]])

    def mlp_attn():
        t1, t2 = [], []

        def act(j, c, toks, u, gs, i0, is_):
            bias = [b1_s[:, cs(j + NF4 * q)] for q in range(4)]
            for n in range(4):
                tk = toks[n * u:]
                ops = _ops2(_lhs_ops,
                            [[_gelu(gate16(c[r][q][n * 16:(n + 1) * 16], tk[gs * (8 * r + 2 * q)],
                                           tk[gs * (8 * r + 2 * q + 1)]) + bias[q])
                              for q in range(4)] for r in range(4)],
                            lambda i, x: gate16(x, tk[i0 + is_ * i], tk[i0 + is_ * i]))
                for p in range(49):
                    a_h[p, j, n * 16:(n + 1) * 16, :] = ops[p].astype(BF16)

        c = None
        for j in range(NF4):
            n0, prev = len(t1), c
            c = _strassen2(lambda p: dot(lhs(ay_u, p, 0, 2), _bf(bw1_u[j, p]), t1))
            if j:
                act(j - 1, prev, t1[n0:], P["gu"], P["gs"], P["gi0"], P["gis"])

        def half(a, p, k0, k1):
            return dot(lhs(ah_u, p, k0, k1), _bf(bw2_u[a, p, k0 * 64:k1 * 64, :]), t2)

        seq = [7 * i + k for i in SORD for k in SORD][:P["ne"]]
        early = {p: half(0, p, 0, 4) for p in seq}
        act(NF4 - 1, c, [t for t in t2 for _ in range(2)], P["hu"], P["hs"], P["hi0"], P["his"])

        def prod2(a, p):
            acc = early[p] if a == 0 and p in early else half(a, p, 0, 4)
            return acc + half(a, p, 4, NF4)

        for a in range(2):
            c = _strassen2(functools.partial(prod2, a))
            done = ((1, 0), (0, 0), (0, 1), (1, 1))
            for ro, qo in done:
                for ri, qi in done:
                    r, q = 2 * ro + ri, 2 * qo + qi
                    cc = a + 2 * q
                    y = (x1_s[r * QM:(r + 1) * QM, cs(cc)] + b2_s[:, cs(cc)]) + c[r][q]
                    xs[pl.ds(prow + r * QM, QM), cs(cc)] = y
                    o_s[pl.ds(prow + r * QM, QM), cs(cc)] = y.astype(BF16)
        ta = t1[:P["a0"]:P["a1"]]
        attn_paced(ta + [t2[P["a3"] + int(n * P["a2"])] for n in range(17 * (NRC + 2) - len(ta))])

    def wq_copy(t):
        return pltpu.make_async_copy(wqkv_hbm.at[:, pl.ds(t * D, D)], wq_raw.at[t], sems.at[t])

    wo_copy = pltpu.make_async_copy(wo_hbm, wo_raw, sems.at[3])

    def mlp_copies(a):
        return [pltpu.make_async_copy(w1_hbm.at[:, a], w1_raw.at[:, a], sems.at[4 + a]),
                pltpu.make_async_copy(w2_hbm.at[:, a], w2_raw.at[:, a], sems.at[8 + a])]

    def x_copy(b):
        rows = pl.ds(b * TM if isinstance(b, int) else pl.multiple_of(b * TM, TM), TM)
        return pltpu.make_async_copy(x_hbm.at[rows], x_s.at[rows], sems.at[12 + b])

    def o_copy(b):
        rows = pl.ds(b * TM if isinstance(b, int) else pl.multiple_of(b * TM, TM), TM)
        return pltpu.make_async_copy(o_s.at[rows], o_hbm.at[rows], sems.at[12 + NB + b])

    bias_copies = [pltpu.make_async_copy(b1_hbm, b1_raw, sems.at[12 + 2 * NB]),
                   pltpu.make_async_copy(b2_hbm, b2_raw, sems.at[13 + 2 * NB])]

    def perm_ops(*kd):
        return [o.astype(BF16) for o in _rhs_ops(*[tmp[k, pl.ds(d, H, stride=PAD), :] for k, d in kd])]

    def start_all():
        x_copy(0).start()
        for t in range(3):
            wq_copy(t).start()
        wo_copy.start()
        x_copy(1).start()
        for cp in bias_copies:
            cp.start()
        for a in range(4):
            for cp in mlp_copies(a):
                cp.start()

    @pl.when(jnp.logical_and(s > 1, s < NB))
    def _wait_x():
        x_copy(jnp.minimum(s, NB - 1)).wait()

    @pl.when(s <= 1)
    def _first_ln():
        pl.when(s == 0)(start_all)
        x_copy(jnp.minimum(s, 1)).wait()
        ln_all(resid(True, row0), st1, a_x)

    @pl.when(s == 0)
    def _prologue():
        qkv_s[:, :, 0:HALO, :] = jnp.zeros((3, NC, HALO, 128), F32)
        eye = (jax.lax.broadcasted_iota(jnp.int32, (128, 128), 0)
               == jax.lax.broadcasted_iota(jnp.int32, (128, 128), 1)).astype(BF16)

        def qkv_body(t, carry):
            wq_copy(t).wait()
            for c in range(NC):
                tile = jax.lax.dot_general(eye, wq_raw[t, :, cs(c)], NT, preferred_element_type=F32)
                for k in range(NC):
                    for hh in range(4):
                        tmp[k, (4 * c + hh) * PAD:(4 * c + hh) * PAD + DH, :] = (
                            tile[hh * DH:(hh + 1) * DH, cs(k)])
            for d in range(DH // 2):
                for k in range(4):
                    ops = perm_ops((k, d), (k, d + 16), (k + 4, d), (k + 4, d + 16))
                    for i in range(7):
                        bq[t, d // 4, i, k, (d % 4) * H:(d % 4 + 1) * H, :] = ops[i]
            proj(t, [lhs(ax_u, i) for i in range(7)], [])
            return carry

        jax.lax.fori_loop(0, 3, qkv_body, 0)
        wo_copy.wait()
        for c in range(NC):
            for h in range(H):
                tmp[c, h * PAD:h * PAD + DH, :] = wo_raw[h * DH:(h + 1) * DH, cs(c)].astype(F32)
        for d in range(DH // 2):
            for c in range(4):
                ops = perm_ops((c, d), (c + 4, d), (c, d + 16), (c + 4, d + 16))
                for i in range(7):
                    bo[c, i, d * H:(d + 1) * H, :] = ops[i]

        def attn_body(j, carry):
            r16 = pl.multiple_of(j * 16, 16)
            for r0 in (r16, r16 + RC, HM + r16, HM + r16 + RC):
                e, inv = attn_softmax(attn_qk(r0), r0, True)
                attn_pv(e, inv, r0)
            combine(st1, a_o, j)
            return carry

        jax.lax.fori_loop(0, NRC // 4, attn_body, 0, unroll=P["au"])

    @pl.when(jnp.logical_and(s > 1, s < 2 * NB))
    def _front():
        toks = []
        out_proj(toks)
        ln_all(resid(s < NB, row0), st1, a_x, toks[::P["l1"]], P["l1lag"])
        qkv_s[1:3, :, 0:HALO, :] = qkv_s[1:3, :, TM:TM + HALO, :]
        toks = []
        av = [lhs(ax_u, i) for i in range(7)]
        for t in range(3):
            proj(t, av, toks)
        ln2(toks[P["l20"]::P["l2"]], P["l2lag"])

    @pl.when(jnp.logical_or(s == 1, s == 2 * NB))
    def _front_last():
        @pl.when(s == 2 * NB)
        def _():
            for b in range(NB - 2):
                o_copy(b).wait()

        out_proj([])
        ln2()

    @pl.when(s == 1)
    def _mlp_weights():
        def prep(raw, dst, a, toks):
            rows, nq = raw.shape[2], raw.shape[3] // 512
            for n in range(0, rows, 16):
                r16 = pl.multiple_of(a * rows + n, 16)
                for j in range(nq):
                    tok = next(toks)
                    ops = _ops2(_rhs_ops, [[gate16(raw[r, a, n:n + 16, cs(q * nq + j)].astype(F32),
                                                   tok if r == q else None)
                                            for q in range(4)] for r in range(4)])
                    for p in range(49):
                        dst[j, p, pl.ds(r16, 16), :] = ops[p].astype(BF16)

        def body(a, carry):
            for cp in mlp_copies(a):
                cp.wait()
            av = [lhs(ax_u, i) for i in range(7)]
            toks = []
            for t in range(3):
                proj(t, av, toks, [a])
            toks = iter([None] * P["p0"] + [toks[int(u * P["p1"])] for u in range(56 - P["p0"])])
            prep(w1_raw, bw1, a, toks)
            prep(w2_raw, bw2, a, toks)
            return carry

        for cp in bias_copies:
            cp.wait()
        b1_s[...] = b1_raw[...].astype(F32).reshape(1, F)
        b2_s[...] = b2_raw[...].astype(F32).reshape(1, D)
        qkv_s[1:3, :, 0:HALO, :] = qkv_s[1:3, :, TM:TM + HALO, :]
        jax.lax.fori_loop(0, 4, body, 0)
        for b in range(2, NB):
            x_copy(b).start()

    @pl.when(s > 0)
    def _back():
        mlp_attn()

    @pl.when(s > NB)
    def _store():
        o_copy(jnp.maximum(s - NB - 1, 0)).start()

    @pl.when(s == 2 * NB)
    def _finish():
        for b in range(NB - 2, NB):
            o_copy(b).wait()


def _build(**kw):
    P = dict(a0=404, a1=4, a2=2.85, a3=140, gu=98, gs=2, gi0=66, gis=4, ne=18, hu=68, hs=1, hi0=44, his=3,
             l1=2, l1lag=4, l20=16, l2=7, l2lag=1, l2c=2, au=1, p0=4, p1=6.4, l1dep=9, l2dep=3)
    P.update(kw)
    any_spec = pl.BlockSpec(memory_space=pl.ANY)
    return pl.pallas_call(
        functools.partial(_kernel, P=P),
        grid=(2 * NB + 1,),
        in_specs=[any_spec] * 7,
        out_specs=any_spec,
        out_shape=jax.ShapeDtypeStruct((S, D), BF16),
        scratch_shapes=[
            pltpu.VMEM((S, D), BF16),
            pltpu.VMEM((S, D), BF16),
            pltpu.VMEM((F,), BF16),
            pltpu.VMEM((D,), BF16),
            pltpu.VMEM((1, F), F32),
            pltpu.VMEM((1, D), F32),
            pltpu.VMEM((3, D, D), BF16),
            pltpu.VMEM((D, D), BF16),
            pltpu.VMEM((4, 4, D // 16, F), BF16),
            pltpu.VMEM((4, 4, F // 16, D), BF16),
            pltpu.VMEM((3, 4, 7, 4, 128, 128), BF16),
            pltpu.VMEM((4, 7, 512, 128), BF16),
            pltpu.VMEM((NF4, 49, 256, 128), BF16),
            pltpu.VMEM((2, 49, F // 4, 128), BF16),
            pltpu.VMEM((NC, H * PAD, 128), F32),
            pltpu.VMEM((S, D), F32),
            pltpu.VMEM((TM, D), F32),
            pltpu.VMEM((NC, TM, 128), F32),
            pltpu.VMEM((NC, TM, 128), F32),
            pltpu.VMEM((7, 4, HM, 128), BF16),
            pltpu.VMEM((49, 2, QM, 128), BF16),
            pltpu.VMEM((7, 4, HM, 128), BF16),
            pltpu.VMEM((49, NF4, QM, 128), BF16),
            pltpu.VMEM((3, NC, TM + HALO, 128), F32),
            pltpu.SemaphoreType.DMA((14 + 2 * NB,)),
        ],
        compiler_params=pltpu.CompilerParams(
            dimension_semantics=("arbitrary",), vmem_limit_bytes=120 * 1024 * 1024),
    )


def _call(fn, A_x, A_wqkv, A_wo, B_x, B_w1, B_b1, B_w2, B_b2):
    del B_x
    out = fn(A_x.reshape(S, D), A_wqkv, A_wo, B_w1.reshape(4, 4, D // 16, F), B_b1,
             B_w2.reshape(4, 4, F // 16, D), B_b2)
    return out.reshape(1, S, D)


@jax.jit
def pallas_interleave_layers__sliding_local_dilated__dense_activation_gelu__prompt_kernel(
    A_x: jax.Array,
    A_wqkv: jax.Array,
    A_wo: jax.Array,
    B_x: jax.Array,
    B_w1: jax.Array,
    B_b1: jax.Array,
    B_w2: jax.Array,
    B_b2: jax.Array,
):
    return _call(_build(), A_x, A_wqkv, A_wo, B_x, B_w1, B_b1, B_w2, B_b2)
```

```python
import functools

import jax
import jax.numpy as jnp
import jax.experimental.pallas as pl
import jax.experimental.pallas.tpu as pltpu

S, D, F = 2048, 1024, 3584
H, DH, WIN, DIL = 32, 32, 8, 2
NC = D // 128
HALO = 16
EPS = 1e-5
SCALE = DH ** -0.5
LOG2E = 1.4426950408889634
PAD = DH + 1
F32, BF16, U32 = jnp.float32, jnp.bfloat16, jnp.uint32
TM, RC = 256, 8
HM, QM, NB, NRC = TM // 2, TM // 4, S // TM, TM // RC
NF4 = F // 512
SORD = (0, 3, 1, 6, 4, 2, 5)
NN = (((1,), (0,)), ((), ()))
NT = (((1,), (1,)), ((), ()))


def _gelu(x):
    c = 0.7978845608028654
    t = jnp.tanh(x * (c + (c * 0.044715) * (x * x)))
    hx = 0.5 * x
    return hx + hx * t


def _tree(p):
    return ((p[0] + p[1]) + (p[2] + p[3])) + ((p[4] + p[5]) + (p[6] + p[7]))


def _lhs_ops(a11, a12, a21, a22):
    return [a11 + a22, a21 + a22, a11, a22, a11 + a12, a21 - a11, a12 - a22]


def _rhs_ops(b11, b12, b21, b22):
    return [b11 + b22, b11, b12 - b22, b21 - b11, b22, b11 + b12, b21 + b22]


def _ops2(ops, blk, gate=None):
    outer = [[ops(blk[r][c], blk[r][c + 2], blk[r + 2][c], blk[r + 2][c + 2]) for c in range(2)]
             for r in range(2)]
    g = (lambda i, x: x) if gate is None else gate
    return [o for i in range(7)
            for o in ops(g(i, outer[0][0][i]), outer[0][1][i], outer[1][0][i], g(i, outer[1][1][i]))]


def _bf(u):
    return pltpu.bitcast(u, BF16)


def _strassen(prod):
    m1 = prod(0)
    m4 = prod(3)
    c11 = m1 + m4
    m2 = prod(1)
    c21 = m2 + m4
    c22 = m1 - m2
    c11 = c11 + prod(6)
    m5 = prod(4)
    c11 = c11 - m5
    m3 = prod(2)
    c12 = m3 + m5
    c22 = (c22 + m3) + prod(5)
    return c11, c12, c21, c22


def _strassen2(prod):
    c = _strassen(lambda i: jnp.concatenate(_strassen(lambda k: prod(7 * i + k)), axis=0))
    n = c[0].shape[0] // 4
    return [[c[2 * (r // 2) + q // 2][(2 * (r % 2) + q % 2) * n:(2 * (r % 2) + q % 2 + 1) * n]
             for q in range(4)] for r in range(4)]


def _kernel(x_hbm, wqkv_hbm, wo_hbm, w1_hbm, b1_hbm, w2_hbm, b2_hbm, o_hbm,
            x_s, o_s, b1_raw, b2_raw, b1_s, b2_s,
            wq_raw, wo_raw, w1_raw, w2_raw, bq, bo, bw1, bw2, tmp, xs, x1_s, st1, st2,
            a_x, a_y, a_o, a_h, qkv_s, sems, *, P):
    s = pl.program_id(0)
    bq_u, bo_u, bw1_u, bw2_u, ax_u, ay_u, ao_u, ah_u = (
        r.bitcast(U32) for r in (bq, bo, bw1, bw2, a_x, a_y, a_o, a_h))
    row0 = pl.multiple_of((s % NB) * TM, TM)
    prow = pl.multiple_of(((s + NB - 1) % NB) * TM, TM)
    live = (jax.lax.broadcasted_iota(jnp.int32, (RC, 128), 0) + s) >= 0
    order = [g for j in range(NRC // 4) for g in (2 * j, 2 * j + 1, NRC // 2 + 2 * j, NRC // 2 + 2 * j + 1)]
    order2 = [8 * q + 2 * g + n for g in range(4) for q in range(4) for n in range(2)]
    cs = lambda c: slice(c * 128, (c + 1) * 128)

    def gate(x, tok):
        return x if tok is None else jnp.where(live, x, tok)

    def gate16(x, tok, tok2=None):
        return jnp.concatenate([gate(x[:RC], tok), gate(x[RC:], tok2)], axis=0)

    def lhs(buf, i, k0=0, k1=4):
        return jnp.concatenate([_bf(buf[i, k]) for k in range(k0, k1)], axis=1)

    def dot(a, b, toks, dims=NN):
        r = jax.lax.dot_general(a, b, dims, preferred_element_type=F32)
        toks.extend(r[j * RC:(j + 1) * RC, :] for j in range(r.shape[0] // RC))
        return r

    def combine(src, dst, j, toks=None):
        r16 = j * 16 if isinstance(j, int) else pl.multiple_of(j * 16, 16)
        for c in range(4):
            tok = None if toks is None else toks[c]
            ld = lambda r, cc: src[cc, pl.ds(r + r16, 16), :]
            ops = _lhs_ops(gate16(ld(0, c), tok), ld(0, c + 4), ld(HM, c), gate16(ld(HM, c + 4), tok))
            for i in range(7):
                dst[i, c, pl.ds(r16, 16), :] = ops[i].astype(BF16)

    def combine2(g, kk, toks=None):
        ops = _ops2(_lhs_ops, [[st2[2 * q + kk, QM * r + 16 * g:QM * r + 16 * g + 16, :]
                                for q in range(4)] for r in range(4)],
                    None if toks is None else lambda i, x: gate16(x, toks[i]))
        for p in range(49):
            a_y[p, kk, 16 * g:16 * g + 16, :] = ops[p].astype(BF16)

    def ln_rows(x, dst, r0, toks, chain, dep):
        prev = chain[-dep] if toks[0] is not None and len(chain) >= dep else None
        m = jnp.sum(gate(gate(_tree(x), toks[0]), prev), axis=1, keepdims=True) * (1.0 / D)
        x = [t - m for t in x]
        v = jnp.sum(gate(_tree([t * t for t in x]), toks[1]), axis=1, keepdims=True) * (1.0 / D)
        chain.append(jnp.broadcast_to(jax.lax.rsqrt(v + EPS), (RC, 128)))
        r = gate(chain[-1], toks[2])
        for c in range(NC):
            dst[c, r0:r0 + RC, :] = x[c] * r

    def ln_all(load, stage, dst, toks=None, lag=0):
        chain = []
        for n, g in enumerate(order):
            tk = [None] * 3 if toks is None else [toks[4 * (n + k * lag) + k] for k in range(3)]
            ln_rows([load(g * RC, c) for c in range(NC)], stage, g * RC, tk, chain, P["l1dep"])
            if n % 4 == 3:
                combine(stage, dst, n // 4,
                        None if toks is None else [toks[4 * (n + 1 + c + 2 * lag) + 3] for c in range(4)])

    def resid(first, base):
        def load(r0, c, rows=RC):
            xin = x_s[pl.ds(base + r0, rows), cs(c)].astype(F32)
            if first is True:
                return xin
            return jnp.where(first, xin, xs[pl.ds(base + r0, rows), cs(c)])
        return load

    def proj(t, av, toks, cols=range(4)):
        for a in cols:
            c = _strassen(lambda i: dot(av[i], jnp.concatenate([_bf(bq_u[t, a, i, k]) for k in range(4)], axis=1), toks, NT))
            for k in range(4):
                r = HALO + (k // 2) * HM
                qkv_s[t, a + 4 * (k % 2), r:r + HM, :] = c[k]

    def attn_qk(r0, toks=None):
        q = [qkv_s[0, c, pl.ds(r0 + HALO, RC), :] for c in range(NC)]
        return [gate(_tree([q[c] * qkv_s[1, c, pl.ds(r0 + HALO - DIL * w, RC), :] for c in range(NC)]),
                     None if toks is None else toks[w])
                for w in range(WIN)]

    def attn_softmax(lg, r0, masked):
        out = []
        for w, t in enumerate(lg):
            t = t + pltpu.roll(t, 64, 1)
            t = t + pltpu.roll(t, 32, 1)
            if w > 0 and masked:
                pos = row0 + r0 + jax.lax.broadcasted_iota(jnp.int32, (RC, 128), 0)
                t = jnp.where(pos >= DIL * w, t, -1e9 / SCALE)
            out.append(t)
        lg = out
        m = jnp.maximum(jnp.maximum(jnp.maximum(lg[0], lg[1]), jnp.maximum(lg[2], lg[3])),
                        jnp.maximum(jnp.maximum(lg[4], lg[5]), jnp.maximum(lg[6], lg[7])))
        e = [jnp.exp2((t - m) * (SCALE * LOG2E)) for t in lg]
        den = _tree(e)
        inv = pl.reciprocal(den, approx=True)
        inv = inv * (2.0 - den * inv)
        return e, inv

    def attn_pv(e, inv, r0, toks=None):
        for c in range(NC):
            t = _tree([e[w] * qkv_s[2, c, pl.ds(r0 + HALO - DIL * w, RC), :] for w in range(WIN)])
            st1[c, pl.ds(r0, RC), :] = t * gate(inv, None if toks is None else toks[c])

    def attn_paced(toks):
        sm = None
        for n in range(NRC + 2):
            tk = toks[17 * n:17 * (n + 1)]
            if n < NRC:
                lg = attn_qk(order[n] * RC, tk[:8])
            if 0 < n <= NRC:
                attn_pv(*sm, order[n - 1] * RC, tk[8:16])
            if n < NRC:
                sm = attn_softmax(lg, order[n] * RC, order[n] * RC < HALO)
            if n > 1 and n % 4 == 1:
                combine(st1, a_o, n // 4 - 1, [tk[3], tk[7], tk[11], tk[16]])

    def out_proj(toks):
        av = [lhs(ao_u, i) for i in range(7)]
        res = resid(s <= NB, prow)
        for a in range(4):
            c = _strassen(lambda i: dot(av[i], _bf(bo_u[a, i]), toks))
            for k in range(4):
                r, cc = (k // 2) * HM, a + 4 * (k % 2)
                x1_s[r:r + HM, cs(cc)] = res(r, cc, HM) + c[k]

    def ln2(toks=None, lag=0):
        chain = []
        for n, g in enumerate(order2):
            tk = [None] * 3 if toks is None else [toks[4 * (n + k * lag) + k] for k in range(3)]
            ln_rows([x1_s[g * RC:(g + 1) * RC, cs(c)] for c in range(NC)], st2, g * RC, tk, chain, P["l2dep"])
            if n % 8 == 7:
                for kk in range(2):
                    n0 = 4 * (n + 2 * lag + 1) + P["l2c"] * 7 * kk + 1
                    combine2(n // 8, kk, None if toks is None else toks[n0::P["l2c"]])

    def mlp_attn():
        t1, t2 = [], []

        def act(j, c, toks, u, gs, i0, is_):
            bias = [b1_s[:, cs(j + NF4 * q)] for q in range(4)]
            for n in range(4):
                tk = toks[n * u:]
                ops = _ops2(_lhs_ops,
                            [[_gelu(gate16(c[r][q][n * 16:(n + 1) * 16], tk[gs * (8 * r + 2 * q)],
                                           tk[gs * (8 * r + 2 * q + 1)]) + bias[q])
                              for q in range(4)] for r in range(4)],
                            lambda i, x: gate16(x, tk[i0 + is_ * i], tk[i0 + is_ * i]))
                for p in range(49):
                    a_h[p, j, n * 16:(n + 1) * 16, :] = ops[p].astype(BF16)

        c = None
        for j in range(NF4):
            n0, prev = len(t1), c
            c = _strassen2(lambda p: dot(lhs(ay_u, p, 0, 2), _bf(bw1_u[j, p]), t1))
            if j:
                act(j - 1, prev, t1[n0:], P["gu"], P["gs"], P["gi0"], P["gis"])

        def half(a, p, k0, k1):
            return dot(lhs(ah_u, p, k0, k1), _bf(bw2_u[a, p, k0 * 64:k1 * 64, :]), t2)

        seq = [7 * i + k for i in SORD for k in SORD][:P["ne"]]
        early = {p: half(0, p, 0, 4) for p in seq}
        act(NF4 - 1, c, [t for t in t2 for _ in range(2)], P["hu"], P["hs"], P["hi0"], P["his"])

        def prod2(a, p):
            acc = early[p] if a == 0 and p in early else half(a, p, 0, 4)
            return acc + half(a, p, 4, NF4)

        for a in range(2):
            c = _strassen2(functools.partial(prod2, a))
            done = ((1, 0), (0, 0), (0, 1), (1, 1))
            for ro, qo in done:
                for ri, qi in done:
                    r, q = 2 * ro + ri, 2 * qo + qi
                    cc = a + 2 * q
                    y = (x1_s[r * QM:(r + 1) * QM, cs(cc)] + b2_s[:, cs(cc)]) + c[r][q]
                    xs[pl.ds(prow + r * QM, QM), cs(cc)] = y
                    o_s[pl.ds(prow + r * QM, QM), cs(cc)] = y.astype(BF16)
        ta = t1[:P["a0"]:P["a1"]]
        attn_paced(ta + [t2[P["a3"] + int(n * P["a2"])] for n in range(17 * (NRC + 2) - len(ta))])

    def wq_copy(t):
        return pltpu.make_async_copy(wqkv_hbm.at[:, pl.ds(t * D, D)], wq_raw.at[t], sems.at[t])

    wo_copy = pltpu.make_async_copy(wo_hbm, wo_raw, sems.at[3])

    def mlp_copies(a):
        return [pltpu.make_async_copy(w1_hbm.at[:, a], w1_raw.at[:, a], sems.at[4 + a]),
                pltpu.make_async_copy(w2_hbm.at[:, a], w2_raw.at[:, a], sems.at[8 + a])]

    def x_copy(b):
        rows = pl.ds(b * TM if isinstance(b, int) else pl.multiple_of(b * TM, TM), TM)
        return pltpu.make_async_copy(x_hbm.at[rows], x_s.at[rows], sems.at[12 + b])

    def o_copy(b):
        rows = pl.ds(b * TM if isinstance(b, int) else pl.multiple_of(b * TM, TM), TM)
        return pltpu.make_async_copy(o_s.at[rows], o_hbm.at[rows], sems.at[12 + NB + b])

    bias_copies = [pltpu.make_async_copy(b1_hbm, b1_raw, sems.at[12 + 2 * NB]),
                   pltpu.make_async_copy(b2_hbm, b2_raw, sems.at[13 + 2 * NB])]

    def perm_ops(*kd):
        return [o.astype(BF16) for o in _rhs_ops(*[tmp[k, pl.ds(d, H, stride=PAD), :] for k, d in kd])]

    def start_all():
        x_copy(0).start()
        for t in range(3):
            wq_copy(t).start()
        wo_copy.start()
        x_copy(1).start()
        for cp in bias_copies:
            cp.start()
        for a in range(4):
            for cp in mlp_copies(a):
                cp.start()

    @pl.when(jnp.logical_and(s > 1, s < NB))
    def _wait_x():
        x_copy(jnp.minimum(s, NB - 1)).wait()

    @pl.when(s <= 1)
    def _first_ln():
        pl.when(s == 0)(start_all)
        x_copy(jnp.minimum(s, 1)).wait()
        ln_all(resid(True, row0), st1, a_x)

    @pl.when(s == 0)
    def _prologue():
        qkv_s[:, :, 0:HALO, :] = jnp.zeros((3, NC, HALO, 128), F32)
        eye = (jax.lax.broadcasted_iota(jnp.int32, (128, 128), 0)
               == jax.lax.broadcasted_iota(jnp.int32, (128, 128), 1)).astype(BF16)

        def qkv_body(t, carry):
            wq_copy(t).wait()
            for c in range(NC):
                tile = jax.lax.dot_general(eye, wq_raw[t, :, cs(c)], NT, preferred_element_type=F32)
                for k in range(NC):
                    for hh in range(4):
                        tmp[k, (4 * c + hh) * PAD:(4 * c + hh) * PAD + DH, :] = (
                            tile[hh * DH:(hh + 1) * DH, cs(k)])
            for d in range(DH // 2):
                for k in range(4):
                    ops = perm_ops((k, d), (k, d + 16), (k + 4, d), (k + 4, d + 16))
                    for i in range(7):
                        bq[t, d // 4, i, k, (d % 4) * H:(d % 4 + 1) * H, :] = ops[i]
            proj(t, [lhs(ax_u, i) for i in range(7)], [])
            return carry

        jax.lax.fori_loop(0, 3, qkv_body, 0)
        wo_copy.wait()

        def wo_fill(n, carry):
            for hh in range(4):
                h = n * 4 + hh
                for c in range(NC):
                    tmp[c, pl.ds(h * PAD, DH), :] = (
                        wo_raw[pl.ds(pl.multiple_of(h * DH, DH), DH), cs(c)].astype(F32))
            return carry

        def wo_ops(n, carry):
            for dd in range(2):
                d = n * 2 + dd
                for c in range(4):
                    ops = perm_ops((c, d), (c + 4, d), (c, d + 16), (c + 4, d + 16))
                    for i in range(7):
                        bo[c, i, pl.ds(pl.multiple_of(d * H, H), H), :] = ops[i]
            return carry

        jax.lax.fori_loop(0, H // 4, wo_fill, 0)
        jax.lax.fori_loop(0, DH // 4, wo_ops, 0)

        def attn_body(j, carry):
            r16 = pl.multiple_of(j * 16, 16)
            for r0 in (r16, r16 + RC, HM + r16, HM + r16 + RC):
                e, inv = attn_softmax(attn_qk(r0), r0, True)
                attn_pv(e, inv, r0)
            combine(st1, a_o, j)
            return carry

        jax.lax.fori_loop(0, NRC // 4, attn_body, 0, unroll=P["au"])

    @pl.when(jnp.logical_and(s > 1, s < 2 * NB))
    def _front():
        toks = []
        out_proj(toks)
        ln_all(resid(s < NB, row0), st1, a_x, toks[::P["l1"]], P["l1lag"])
        qkv_s[1:3, :, 0:HALO, :] = qkv_s[1:3, :, TM:TM + HALO, :]
        toks = []
        av = [lhs(ax_u, i) for i in range(7)]
        for t in range(3):
            proj(t, av, toks)
        ln2(toks[P["l20"]::P["l2"]], P["l2lag"])

    @pl.when(jnp.logical_or(s == 1, s == 2 * NB))
    def _front_last():
        @pl.when(s == 2 * NB)
        def _():
            for b in range(NB - 2):
                o_copy(b).wait()

        out_proj([])
        ln2()

    @pl.when(s == 1)
    def _mlp_weights():
        def prep(raw, dst, a, toks):
            rows, nq = raw.shape[2], raw.shape[3] // 512
            for n in range(0, rows, 16):
                r16 = pl.multiple_of(a * rows + n, 16)
                for j in range(nq):
                    tok = next(toks)
                    ops = _ops2(_rhs_ops, [[gate16(raw[r, a, n:n + 16, cs(q * nq + j)].astype(F32),
                                                   tok if r == q else None)
                                            for q in range(4)] for r in range(4)])
                    for p in range(49):
                        dst[j, p, pl.ds(r16, 16), :] = ops[p].astype(BF16)

        def body(a, carry):
            for cp in mlp_copies(a):
                cp.wait()
            av = [lhs(ax_u, i) for i in range(7)]
            toks = []
            for t in range(3):
                proj(t, av, toks, [a])
            toks = iter([None] * P["p0"] + [toks[int(u * P["p1"])] for u in range(56 - P["p0"])])
            prep(w1_raw, bw1, a, toks)
            prep(w2_raw, bw2, a, toks)
            return carry

        for cp in bias_copies:
            cp.wait()
        b1_s[...] = b1_raw[...].astype(F32).reshape(1, F)
        b2_s[...] = b2_raw[...].astype(F32).reshape(1, D)
        qkv_s[1:3, :, 0:HALO, :] = qkv_s[1:3, :, TM:TM + HALO, :]
        jax.lax.fori_loop(0, 4, body, 0)
        for b in range(2, NB):
            x_copy(b).start()

    @pl.when(s > 0)
    def _back():
        mlp_attn()

    @pl.when(s > NB)
    def _store():
        o_copy(jnp.maximum(s - NB - 1, 0)).start()

    @pl.when(s == 2 * NB)
    def _finish():
        for b in range(NB - 2, NB):
            o_copy(b).wait()


def _build(**kw):
    P = dict(a0=404, a1=4, a2=2.85, a3=140, gu=98, gs=2, gi0=66, gis=4, ne=18, hu=68, hs=1, hi0=44, his=3,
             l1=2, l1lag=4, l20=16, l2=7, l2lag=1, l2c=2, au=1, p0=4, p1=6.4, l1dep=9, l2dep=3)
    P.update(kw)
    any_spec = pl.BlockSpec(memory_space=pl.ANY)
    return pl.pallas_call(
        functools.partial(_kernel, P=P),
        grid=(2 * NB + 1,),
        in_specs=[any_spec] * 7,
        out_specs=any_spec,
        out_shape=jax.ShapeDtypeStruct((S, D), BF16),
        scratch_shapes=[
            pltpu.VMEM((S, D), BF16),
            pltpu.VMEM((S, D), BF16),
            pltpu.VMEM((F,), BF16),
            pltpu.VMEM((D,), BF16),
            pltpu.VMEM((1, F), F32),
            pltpu.VMEM((1, D), F32),
            pltpu.VMEM((3, D, D), BF16),
            pltpu.VMEM((D, D), BF16),
            pltpu.VMEM((4, 4, D // 16, F), BF16),
            pltpu.VMEM((4, 4, F // 16, D), BF16),
            pltpu.VMEM((3, 4, 7, 4, 128, 128), BF16),
            pltpu.VMEM((4, 7, 512, 128), BF16),
            pltpu.VMEM((NF4, 49, 256, 128), BF16),
            pltpu.VMEM((2, 49, F // 4, 128), BF16),
            pltpu.VMEM((NC, H * PAD, 128), F32),
            pltpu.VMEM((S, D), F32),
            pltpu.VMEM((TM, D), F32),
            pltpu.VMEM((NC, TM, 128), F32),
            pltpu.VMEM((NC, TM, 128), F32),
            pltpu.VMEM((7, 4, HM, 128), BF16),
            pltpu.VMEM((49, 2, QM, 128), BF16),
            pltpu.VMEM((7, 4, HM, 128), BF16),
            pltpu.VMEM((49, NF4, QM, 128), BF16),
            pltpu.VMEM((3, NC, TM + HALO, 128), F32),
            pltpu.SemaphoreType.DMA((14 + 2 * NB,)),
        ],
        compiler_params=pltpu.CompilerParams(
            dimension_semantics=("arbitrary",), vmem_limit_bytes=120 * 1024 * 1024),
    )


def _call(fn, A_x, A_wqkv, A_wo, B_x, B_w1, B_b1, B_w2, B_b2):
    del B_x
    out = fn(A_x.reshape(S, D), A_wqkv, A_wo, B_w1.reshape(4, 4, D // 16, F), B_b1,
             B_w2.reshape(4, 4, F // 16, D), B_b2)
    return out.reshape(1, S, D)


@jax.jit
def pallas_interleave_layers__sliding_local_dilated__dense_activation_gelu__prompt_kernel(
    A_x: jax.Array,
    A_wqkv: jax.Array,
    A_wo: jax.Array,
    B_x: jax.Array,
    B_w1: jax.Array,
    B_b1: jax.Array,
    B_w2: jax.Array,
    B_b2: jax.Array,
):
    return _call(_build(), A_x, A_wqkv, A_wo, B_x, B_w1, B_b1, B_w2, B_b2)
```
